```python
import jax
import jax.numpy as jnp

def _softmax(x, axis=-1):
    return jax.nn.softmax(x, axis=axis)

def _gelu(x):
    return jax.nn.gelu(x, approximate=True)

def _silu(x):
    return jax.nn.silu(x)

def _sigmoid(x):
    return jax.nn.sigmoid(x)

def _layernorm(x, axis=-1, eps=1e-05):
    m = jnp.mean(x, axis=axis, keepdims=True)
    v = jnp.var(x, axis=axis, keepdims=True)
    return (x - m) / jnp.sqrt(v + eps)

def _scatter_add(tgt, idx, src, axis=0):
    return tgt.at[idx].add(src)

def _segment_sum(src, seg, n):
    return jax.ops.segment_sum(src, seg, n)

class _Rng:

    def __init__(self, key):
        self._k = key

    def _next(self):
        self._k, sub = jax.random.split(self._k)
        return sub

    def normal(self, shape):
        return jax.random.normal(self._next(), shape, dtype=jnp.bfloat16)

    def randint(self, lo, hi, shape):
        return jax.random.randint(self._next(), shape, lo, hi, dtype=jnp.int32)

    def uniform(self, shape, lo=0.0, hi=1.0):
        return jax.random.uniform(self._next(), shape, jnp.bfloat16, lo, hi)

    def permutation(self, n):
        return jax.random.permutation(self._next(), n)
kernel_name = 'concat_heads__memory_aug_recurrent_mem_tr__sliding_local_dilated__prompt'

def setup_inputs():
    _rng = _Rng(jax.random.key(int.from_bytes(__import__("os").urandom(4), "little")))
    _w = lambda a: (lambda t: t.astype(jnp.bfloat16) if jnp.issubdtype(t.dtype, jnp.floating) else t)(jnp.asarray(a))

    def _A_setup():
        B, S, Dm = (1, 2048, 1024)
        H, Dh = (32, 128)
        M, seg = (8, 32)
        seg = min(seg, S)
        S = S // seg * seg
        return {'x': _w((lambda *s: _rng.normal(s) * 0.05)(B, S, Dm)), 'mem0': _w((lambda *s: _rng.normal(s) * 0.05)(B, M, Dm)), 'Wq': _w((lambda *s: _rng.normal(s) * 0.05)(Dm, H, Dh) * Dm ** (-0.5)), 'Wk': _w((lambda *s: _rng.normal(s) * 0.05)(Dm, H, Dh) * Dm ** (-0.5)), 'Wv': _w((lambda *s: _rng.normal(s) * 0.05)(Dm, H, Dh) * Dm ** (-0.5)), 'Wo': _w((lambda *s: _rng.normal(s) * 0.05)(H, Dh, Dm) * (H * Dh) ** (-0.5)), 'seg_len': seg}
    _A_in = _A_setup()

    def _B_setup():
        B, S, D = (1, 2048, 1024)
        return {'x': _w((lambda *s: _rng.normal(s) * 0.05)(B, S, D)), 'wqkv': _w((lambda *s: _rng.normal(s) * 0.05)(D, 3 * D)), 'wo': _w((lambda *s: _rng.normal(s) * 0.05)(D, D))}
    _B_in = _B_setup()
    return {'A_x': _A_in['x'], 'A_mem0': _A_in['mem0'], 'A_Wq': _A_in['Wq'], 'A_Wk': _A_in['Wk'], 'A_Wv': _A_in['Wv'], 'A_Wo': _A_in['Wo'], 'A_seg_len': _A_in['seg_len'], 'B_x': _B_in['x'], 'B_wqkv': _B_in['wqkv'], 'B_wo': _B_in['wo']}

def reference(A_x, A_mem0, A_Wq, A_Wk, A_Wv, A_Wo, A_seg_len, B_x, B_wqkv, B_wo):

    def _A_ref(x, mem0, Wq, Wk, Wv, Wo, seg_len):
        B, S, Dm = x.shape
        H, Dh = (Wq.shape[1], Wq.shape[2])
        M = mem0.shape[1]
        scale = Dh ** (-0.5)
        n_seg = S // seg_len
        L = M + seg_len
        idx = jnp.arange(L)
        mask = (idx[:, None] < M) | (idx[:, None] >= idx[None, :])
        mem = mem0
        outs = []
        for s in range(n_seg):
            xs = x[:, s * seg_len:(s + 1) * seg_len, :].copy()
            h = jnp.concatenate([mem, xs], axis=1)
            q = jnp.einsum('btd,dhe->bhte', h, Wq)
            k = jnp.einsum('btd,dhe->bhte', h, Wk)
            v = jnp.einsum('btd,dhe->bhte', h, Wv)
            scores = jnp.einsum('bhqe,bhke->bhqk', q, k) * scale
            scores = jnp.where(mask[None, None], scores, -1000000000.0)
            p = _softmax(scores, axis=-1)
            o = jnp.einsum('bhqk,bhke->bhqe', p, v)
            o = jnp.einsum('bhte,hed->btd', o, Wo)
            mem = o[:, :M, :].copy()
            outs.append(o[:, M:, :])
        return jnp.concatenate(outs, axis=1)

    def _B_ref(x, wqkv, wo):
        B, S, D = x.shape
        H = 32
        Dh = D // H
        W, dil = (8, 2)
        qkv = (lambda x, *d: x.transpose(*d))((x @ wqkv).reshape(B, S, 3, H, Dh), 2, 0, 3, 1, 4)
        q, k, v = (qkv[0], qkv[1], qkv[2])
        scale = Dh ** (-0.5)
        pos = jnp.arange(S)
        off = jnp.arange(W) * dil
        idx = pos[:, None] - off[None, :]
        mask = idx >= 0
        idx_c = jnp.where(mask, idx, 0).reshape(-1)
        kg = k[:, :, idx_c, :].reshape(B, H, S, W, Dh)
        vg = v[:, :, idx_c, :].reshape(B, H, S, W, Dh)
        logits = jnp.einsum('bhsd,bhswd->bhsw', q, kg) * scale
        logits = jnp.where(mask[None, None, :, :], logits, -1000000000.0)
        attn = _softmax(logits, axis=-1)
        o = jnp.einsum('bhsw,bhswd->bhsd', attn, vg)
        return (lambda x, *d: x.transpose(*d))(o, 0, 2, 1, 3).reshape(B, S, D) @ wo
    a = _A_ref(A_x, A_mem0, A_Wq, A_Wk, A_Wv, A_Wo, A_seg_len)
    b = _B_ref(B_x, B_wqkv, B_wo)
    return jnp.concatenate([a, b], axis=-1)
```

```python
import functools

import jax
import jax.numpy as jnp
from jax import lax
import jax.experimental.pallas as pl
import jax.experimental.pallas.tpu as pltpu

LANES = 128
NEG = -1000000000.0

B_HEADS = 32
B_TAPS = 8
B_DIL = 2
B_PAD = 16

A_GROUP = 4
A_UNROLL = 4
KV_ROWS = 512
QO_ROWS = 256
QO_SUB = 128

F32 = jnp.float32
BF16 = jnp.bfloat16
U32 = jnp.uint32


def _dot(a, b):
    return jnp.dot(a, b, preferred_element_type=F32)


def _dot_nt(a, b):
    return lax.dot_general(a, b, (((1,), (1,)), ((), ())), preferred_element_type=F32)


def _bf16(words):
    return pltpu.bitcast(words, BF16)


def _words(halves):
    return pltpu.bitcast(halves, U32)


def _swap_blocks(xs, axis, unit):
    xs = list(xs)
    size = xs[0].shape[axis]
    pos = lax.broadcasted_iota(jnp.int32, xs[0].shape, axis)
    k = 1
    while k < len(xs):
        low = (pos & (k * unit)) == 0
        for t in range(len(xs)):
            if t & k == 0:
                a, b = xs[t], xs[t + k]
                xs[t] = jnp.where(low, a, pltpu.roll(b, k * unit, axis))
                xs[t + k] = jnp.where(low, pltpu.roll(a, size - k * unit, axis), b)
        k *= 2
    return xs


def _kernel(
    xa_hbm, mem_hbm, wq_hbm, wk_hbm, wv_hbm, woa_hbm, xb_hbm, wqkv_hbm, wob_hbm,
    out_hbm,
    wq, wk, wv, woa, wqkv, wob,
    wq_raw, wk_raw, wv_raw, woa_raw, wqkv_raw, wob_raw,
    xa, xb, mem_raw, mem, kb, vb, oa, ob,
    sems,
    *, seg,
):
    S, D = xa.shape
    _, H, DH = wq_raw.shape
    M = mem.shape[0]
    L = M + seg
    pitch = D // 2 + 1
    n_tiles = D // LANES
    n_kv = S // KV_ROWS
    n_qo = S // QO_ROWS

    sem_ids = iter(range(sems.shape[0]))

    def chunked_copy(src, dst, n, cols=None):
        rows = src.shape[0] // n
        base = next(sem_ids)
        for _ in range(n - 1):
            next(sem_ids)

        def copy(i):
            r = i * rows if isinstance(i, int) else pl.multiple_of(i * rows, rows)
            idx = (pl.ds(r, rows),) if cols is None else (pl.ds(r, rows), cols)
            return pltpu.make_async_copy(src.at[idx], dst.at[idx], sems.at[base + i])

        return copy

    q_cols, k_cols, v_cols = (slice(i * D, (i + 1) * D) for i in range(3))
    xb_copy = chunked_copy(xb_hbm, xb, n_kv)
    bk_copy = chunked_copy(wqkv_hbm, wqkv_raw, n_kv, k_cols)
    bv_copy = chunked_copy(wqkv_hbm, wqkv_raw, n_kv, v_cols)
    bq_copy = chunked_copy(wqkv_hbm, wqkv_raw, n_kv, q_cols)
    bo_copy = chunked_copy(wob_hbm, wob_raw, 1)
    ao_copy = chunked_copy(woa_hbm, woa_raw, n_kv)
    aq_copy = chunked_copy(wq_hbm, wq_raw, n_kv)
    ak_copy = chunked_copy(wk_hbm, wk_raw, n_qo)
    av_copy = chunked_copy(wv_hbm, wv_raw, n_qo)
    xa_copy = chunked_copy(xa_hbm, xa, 1)
    mem_copy = chunked_copy(mem_hbm, mem_raw, 1)
    oa_sem = sems.at[next(sem_ids)]
    ob_sem = sems.at[next(sem_ids)]

    def pack_b_cols(i, cols):
        rows = D // n_kv
        for r in range(0, rows, 64):
            src = pl.ds(pl.multiple_of(i * rows + r, 64), 64)
            dst = pl.ds(pl.multiple_of((i * rows + r) // 2, 32), 32)
            xs = [
                _words(wqkv_raw[src, pl.ds(cols.start + t * LANES, LANES)])
                for t in range(n_tiles)
            ]
            for j, x in enumerate(_swap_blocks(xs, 1, 4)):
                wqkv[dst, pl.ds(cols.start + j * LANES, LANES)] = x

    def pack_b_out(i):
        width = D // n_kv
        cols = pl.ds(pl.multiple_of(i * width, width), width)
        for g in range(4):
            for th in range(2):
                for jh in range(2):
                    xs = [
                        _words(wob_raw[pl.ds((4 * th + t) * 128 + g * 32 + jh * 16, 16), cols])
                        for t in range(4)
                    ]
                    for j, x in enumerate(_swap_blocks(xs, 0, 2)):
                        wob[pl.ds((4 * jh + j) * 64 + g * 16 + th * 8, 8), cols] = x

    def pack_a_heads(raw, dst, i, n):
        rows = D // n
        for r in range(0, rows, 2):
            a = _words(raw[i * rows + r])
            b = _words(raw[i * rows + r + 1])
            at = (i * rows + r) // 2
            dst[pl.ds(at, H // 2, stride=pitch), :] = (a & 0xFFFF) | (b << 16)
            dst[pl.ds(H // 2 * pitch + at, H // 2, stride=pitch), :] = (a >> 16) | (
                b & jnp.uint32(0xFFFF0000)
            )

    def pack_a_out(i):
        rows = H * DH // n_kv
        for r in range(0, rows, 128):
            src = pl.ds(pl.multiple_of(i * rows + r, 128), 128)
            dst = pl.ds(pl.multiple_of((i * rows + r) // 2, 64), 64)
            woa[dst, :] = _words(woa_raw[src, :])

    def project_to(dst, i, cols):
        r0 = pl.multiple_of(i * KV_ROWS, KV_ROWS)
        y = _dot(xb[pl.ds(r0, KV_ROWS), :], _bf16(wqkv[:, cols]))
        for t in range(n_tiles):
            dst[t, pl.ds(B_PAD + r0, KV_ROWS), :] = y[:, t * LANES:(t + 1) * LANES]

    def k_step(i, carry):
        xb_copy(i).wait()
        bv_copy(i).wait()
        bq_copy(i).wait()
        project_to(kb, i, k_cols)
        pack_b_cols(i, v_cols)
        pack_b_cols(i, q_cols)
        return carry

    def v_step(i, carry):
        ao_copy(i).wait()
        aq_copy(i).wait()
        project_to(vb, i, v_cols)
        pack_b_out(i)
        pack_a_out(i)
        pack_a_heads(wq_raw, wq, i, n_kv)
        return carry

    def window_attention(q, r0):
        scale = (D // B_HEADS) ** -0.5
        lane = lax.broadcasted_iota(jnp.int32, (8, LANES), 1)
        row = lax.broadcasted_iota(jnp.int32, (8, LANES), 0)
        odd1 = (lane & 1) != 0
        odd2 = (lane & 2) != 0
        out = []
        for r in range(0, q.shape[0], 8):
            qs = [q[r:r + 8, t * LANES:(t + 1) * LANES] for t in range(n_tiles)]
            taps = [pl.ds(B_PAD + r0 + r - B_DIL * w, 8) for w in range(B_TAPS)]
            logits = []
            for w, tap in enumerate(taps):
                x = qs[0] * kb[0, tap, :]
                for t in range(1, n_tiles):
                    x = x + qs[t] * kb[t, tap, :]
                x = x + jnp.where(odd1, pltpu.roll(x, 1, 1), pltpu.roll(x, LANES - 1, 1))
                x = x + jnp.where(odd2, pltpu.roll(x, 2, 1), pltpu.roll(x, LANES - 2, 1))
                x = x * scale
                if w:
                    x = jnp.where(row + (r0 + r) >= B_DIL * w, x, NEG)
                logits.append(x)
            top = functools.reduce(jnp.maximum, logits)
            e = [jnp.exp(x - top) for x in logits]
            inv = 1.0 / functools.reduce(jnp.add, e)
            p = [x * inv for x in e]
            tiles = []
            for t in range(n_tiles):
                o = p[0] * vb[t, taps[0], :]
                for w in range(1, B_TAPS):
                    o = o + p[w] * vb[t, taps[w], :]
                tiles.append(o)
            out.append(jnp.concatenate(tiles, axis=1))
        return jnp.concatenate(out, axis=0).astype(BF16)

    def qo_step(i, carry):
        ak_copy(i).wait()
        av_copy(i).wait()
        r0 = pl.multiple_of(i * QO_ROWS, QO_ROWS)
        starts = [r0 + r for r in range(0, QO_ROWS, QO_SUB)]
        qs = [_dot(xb[pl.ds(r, QO_SUB), :], _bf16(wqkv[:, q_cols])) for r in starts]
        for q, r in zip(qs, starts):
            o = window_attention(q, r)
            ob[pl.ds(r, QO_SUB), :] = _dot(o, _bf16(wob[...])).astype(BF16)
        pack_a_heads(wk_raw, wk, i, n_qo)
        pack_a_heads(wv_raw, wv, i, n_qo)
        rows = pl.ds(r0, QO_ROWS)
        pltpu.make_async_copy(ob.at[rows], out_hbm.at[rows, pl.ds(D, D)], ob_sem).start()
        return carry

    xb_copy(0).start()
    for i in range(n_kv):
        bk_copy(i).start()
    for i in range(n_kv):
        bv_copy(i).start()
        bq_copy(i).start()
        if i + 1 < n_kv:
            xb_copy(i + 1).start()
    bo_copy(0).start()
    for i in range(n_kv):
        ao_copy(i).start()
        aq_copy(i).start()
    for i in range(n_qo):
        ak_copy(i).start()
        av_copy(i).start()
    mem_copy(0).start()
    xa_copy(0).start()

    for t in range(n_tiles):
        kb[t, 0:B_PAD, :] = jnp.zeros((B_PAD, LANES), F32)
    for i in range(n_kv):
        bk_copy(i).wait()
        pack_b_cols(i, k_cols)
    lax.fori_loop(0, n_kv, k_step, 0)
    bo_copy(0).wait()
    lax.fori_loop(0, n_kv, v_step, 0)
    for t in range(n_tiles):
        vb[t, 0:B_PAD, :] = jnp.broadcast_to(vb[t, B_PAD:B_PAD + 1, :], (B_PAD, LANES))
    lax.fori_loop(0, n_qo, qo_step, 0)

    def head_weights(w, g, lo=0, hi=D):
        slots = [(h % 2) * (H // 2) + h // 2 for h in range(g * A_GROUP, (g + 1) * A_GROUP)]
        return jnp.concatenate(
            [_bf16(w[pl.ds(s * pitch + lo // 2, (hi - lo) // 2), :]) for s in slots], axis=1
        )

    def segment(s, memory):
        scale = DH ** -0.5
        row = lax.broadcasted_iota(jnp.int32, (L, L), 0)
        col = lax.broadcasted_iota(jnp.int32, (L, L), 1)
        mask = (row < M) | (row >= col)
        rows = pl.ds(pl.multiple_of(s * seg, seg), seg)
        h = jnp.concatenate([memory, xa[rows, :].astype(F32)], axis=0)
        heads = [slice(j * DH, (j + 1) * DH) for j in range(A_GROUP)]

        def project(g):
            return tuple(_dot(h, head_weights(w, g)) for w in (wq, wk, wv))

        def scores(qkv):
            q, k, _ = qkv
            return [_dot_nt(q[:, c], k[:, c]) for c in heads]

        def attend(sc, qkv):
            out = []
            for x, c in zip(sc, heads):
                x = jnp.where(mask, x * scale, NEG)
                e = jnp.exp(x - jnp.max(x, axis=-1, keepdims=True))
                p = e / jnp.sum(e, axis=-1, keepdims=True)
                out.append(_dot(p, qkv[2][:, c]))
            return out

        q0 = _dot(h[:, :D // 2], head_weights(wq, 0, 0, D // 2))
        q0 = _dot(h[:, D // 2:], head_weights(wq, 0, D // 2, D)) + q0
        qkv = (q0, _dot(h, head_weights(wk, 0)), _dot(h, head_weights(wv, 0)))
        u = []
        for g in range(1, H // A_GROUP):
            sc = scores(qkv)
            nxt = project(g)
            u += attend(sc, qkv)
            qkv = nxt
        sc = scores(qkv)
        split = H // 2
        o = _dot(jnp.concatenate(u[:split], axis=1), _bf16(woa[:split * DH // 2, :]))
        u += attend(sc, qkv)
        o = _dot(jnp.concatenate(u[split:], axis=1), _bf16(woa[split * DH // 2:, :])) + o
        oa[rows, :] = o[M:].astype(BF16)
        return o[:M]

    def a_step(i, carry):
        memory = mem[...]
        for j in range(A_UNROLL):
            memory = segment(i * A_UNROLL + j, memory)
        mem[...] = memory
        n = A_UNROLL * seg
        rows = pl.ds(pl.multiple_of(i * n, n), n)
        pltpu.make_async_copy(oa.at[rows], out_hbm.at[rows, pl.ds(0, D)], oa_sem).start()
        return carry

    mem_copy(0).wait()
    xa_copy(0).wait()
    mem[...] = mem_raw[...].astype(F32)
    lax.fori_loop(0, S // seg // A_UNROLL, a_step, 0)

    pltpu.make_async_copy(ob, out_hbm.at[:, pl.ds(D, D)], ob_sem).wait()
    pltpu.make_async_copy(oa, out_hbm.at[:, pl.ds(0, D)], oa_sem).wait()


@functools.partial(jax.jit, static_argnames=("A_seg_len",))
def pallas_concat_heads__memory_aug_recurrent_mem_tr__sliding_local_dilated__prompt_kernel(
    A_x: jax.Array,
    A_mem0: jax.Array,
    A_Wq: jax.Array,
    A_Wk: jax.Array,
    A_Wv: jax.Array,
    A_Wo: jax.Array,
    A_seg_len: int,
    B_x: jax.Array,
    B_wqkv: jax.Array,
    B_wo: jax.Array,
):
    batch, S, D = A_x.shape
    _, H, DH = A_Wq.shape
    M = A_mem0.shape[1]
    seg = int(A_seg_len)
    assert batch == 1 and B_x.shape == A_x.shape
    assert DH == LANES and D == 8 * LANES and D // B_HEADS == 32
    assert S % (seg * A_UNROLL) == 0 and S % KV_ROWS == 0 and S % QO_ROWS == 0

    head_words = pltpu.VMEM((H * (D // 2 + 1), DH), U32)
    head_raw = pltpu.VMEM((D, H, DH), BF16)
    tokens = pltpu.VMEM((S, D), BF16)
    window = pltpu.VMEM((D // LANES, B_PAD + S, LANES), F32)
    n_sems = 6 * (S // KV_ROWS) + 2 * (S // QO_ROWS) + 5

    out = pl.pallas_call(
        functools.partial(_kernel, seg=seg),
        out_shape=jax.ShapeDtypeStruct((S, 2 * D), BF16),
        in_specs=[pl.BlockSpec(memory_space=pl.ANY)] * 9,
        out_specs=pl.BlockSpec(memory_space=pl.ANY),
        scratch_shapes=[
            head_words, head_words, head_words,
            pltpu.VMEM((H * DH // 2, D), U32),
            pltpu.VMEM((D // 2, 3 * D), U32),
            pltpu.VMEM((D // 2, D), U32),
            head_raw, head_raw, head_raw,
            pltpu.VMEM((H * DH, D), BF16),
            pltpu.VMEM((D, 3 * D), BF16),
            pltpu.VMEM((D, D), BF16),
            tokens, tokens,
            pltpu.VMEM((M, D), BF16),
            pltpu.VMEM((M, D), F32),
            window, window,
            tokens, tokens,
            pltpu.SemaphoreType.DMA((n_sems,)),
        ],
        compiler_params=pltpu.CompilerParams(vmem_limit_bytes=126 * 1024 * 1024),
        name="concat_heads",
    )(
        A_x.reshape(S, D), A_mem0.reshape(M, D), A_Wq, A_Wk, A_Wv,
        A_Wo.reshape(H * DH, D), B_x.reshape(S, D), B_wqkv, B_wo,
    )
    return out.reshape(batch, S, 2 * D)
```

```python
import functools

import jax
import jax.numpy as jnp
from jax import lax
import jax.experimental.pallas as pl
import jax.experimental.pallas.tpu as pltpu

LANES = 128
NEG = -1000000000.0

B_HEADS = 32
B_TAPS = 8
B_DIL = 2
B_PAD = 16

A_GROUP = 4
A_UNROLL = 2
A_PASS = 32
ROWS = 512
SKEW = 8

F32 = jnp.float32
BF16 = jnp.bfloat16
U32 = jnp.uint32
I32 = jnp.int32


def _dot(a, b):
    return jnp.dot(a, b, preferred_element_type=F32)


def _dot_nt(a, b):
    return lax.dot_general(a, b, (((1,), (1,)), ((), ())), preferred_element_type=F32)


def _bf16(words):
    return pltpu.bitcast(words, BF16)


def _words(halves):
    return pltpu.bitcast(halves, U32)


def _rows(start, size, align=None):
    if not isinstance(start, int):
        start = pl.multiple_of(start, size if align is None else align)
    return pl.ds(start, size)


def _add(a, b):
    return (a.astype(F32) + b.astype(F32)).astype(BF16)


def _sub(a, b):
    return (a.astype(F32) - b.astype(F32)).astype(BF16)


def _left_sums(a):
    a11, a12, a21, a22 = a(0, 0), a(0, 1), a(1, 0), a(1, 1)
    return {1: _add(a11, a22), 2: _add(a21, a22), 5: _add(a11, a12),
            6: _sub(a21, a11), 7: _sub(a12, a22)}


def _strassen(left, b, each):
    def product(n, right):
        y = _dot(left(n), right)
        each(y)
        return y

    m5 = product(5, b(1, 1))
    m3 = product(3, _sub(b(0, 1), b(1, 1)))
    c12 = m3 + m5
    c22 = product(6, _add(b(0, 0), b(0, 1))) + m3
    m2 = product(2, b(0, 0))
    c22 = c22 - m2
    c11 = product(7, _add(b(1, 0), b(1, 1))) - m5
    m4 = product(4, _sub(b(1, 0), b(0, 0)))
    c11 = m4 + c11
    c21 = m4 + m2
    m1 = product(1, _add(b(0, 0), b(1, 1)))
    c11 = m1 + c11
    c22 = m1 + c22
    return jnp.concatenate(
        [jnp.concatenate([c11, c12], axis=1), jnp.concatenate([c21, c22], axis=1)], axis=0)


def _swap_blocks(xs, axis, unit, zero):
    n = len(xs)
    size = xs[0].shape[axis]
    pos = ((lax.broadcasted_iota(I32, zero.shape, axis) | zero) // unit) % n
    pos = jnp.tile(pos, (xs[0].shape[0] // zero.shape[0], xs[0].shape[1] // zero.shape[1]))
    xs = [pltpu.roll(x, t * unit, axis) if t else x for t, x in enumerate(xs)]
    out = []
    for j in range(n):
        y = xs[0]
        for t in range(1, n):
            y = jnp.where(pos == (j + t) % n, xs[t], y)
        out.append(y)
    return [pltpu.roll(y, size - j * unit, axis) if j else y for j, y in enumerate(out)]


def _kernel(
    xa_hbm, mem_hbm, wq_hbm, wk_hbm, wv_hbm, woa_hbm, xb_hbm, wqkv_hbm, wob_hbm,
    out_hbm,
    wq, wk, wv, wo, woa_raw, xa, mem_raw, mem, xa_left, kb, vqb, zeros, sems,
    *, seg,
):
    S, D = xa.shape
    _, H, DH = wq_hbm.shape
    M = mem.shape[0]
    L = M + seg
    n_seg = S // seg
    head = A_PASS - M
    rest = seg - head
    pitch = D // 2 + SKEW
    n_tiles = D // LANES
    n_rows = S // ROWS
    n_groups = H // A_GROUP
    n_rest = H * DH // D
    pair = 2 * LANES
    vb, qb = vqb.at[0], vqb.at[1]

    sem_ids = iter(range(sems.shape[0]))

    def chunked_copy(src, dst, n):
        rows = src.shape[0] // n
        base = [next(sem_ids) for _ in range(n)][0]
        return lambda i: pltpu.make_async_copy(
            src.at[_rows(i * rows, rows)], dst.at[_rows(i * rows, rows)], sems.at[base + i])

    ao_copy = chunked_copy(woa_hbm, woa_raw, 1)
    xa_copy = chunked_copy(xa_hbm, xa, 1)
    mem_copy = chunked_copy(mem_hbm, mem_raw, 1)
    oa_sem = sems.at[next(sem_ids)]
    ob_sem = sems.at[next(sem_ids)]
    rest_sem = sems.at[next(sem_ids)]

    def pack_b_cols(raw, dst, first, rows, zero):
        xs = [_words(raw[_rows(first, rows), t * LANES:(t + 1) * LANES])
              for t in range(n_tiles)]
        for j, x in enumerate(_swap_blocks(xs, 1, 4, zero)):
            dst[_rows(first // 2, rows // 2), j * LANES:(j + 1) * LANES] = x

    def pack_b_out(raw, cols, part, zero):
        g, th, jh = part // 4, part // 2 % 2, part % 2
        xs = [_words(raw[pl.ds((4 * th + t) * 128 + g * 32 + jh * 16, 16), cols])
              for t in range(4)]
        for j, x in enumerate(_swap_blocks(xs, 0, 2, zero)):
            wo[pl.ds(H * DH // 2 + (4 * jh + j) * 64 + g * 16 + th * 8, 8), cols] = x

    def pack_a_heads(raw, dst, first, rows, zero):
        half = jnp.tile((zero | 16).astype(U32), (H // 16, 1))
        for r in range(rows // 2):
            at = first // 2 + r
            a = _words(raw[2 * at])
            b = _words(raw[2 * at + 1])
            dst[pl.ds(at, H // 2, stride=pitch), :] = (a & 0xFFFF) | (b << half)
            dst[pl.ds(H // 2 * pitch + at, H // 2, stride=pitch), :] = (a >> half) | (
                b & jnp.uint32(0xFFFF0000))

    def head_weight(w, g, j, lo, hi):
        slot = (j % 2) * (H // 2) + g * (A_GROUP // 2) + j // 2
        return _bf16(w[pl.ds(slot * pitch + lo // 2, (hi - lo) // 2), :])

    def group_weight(w, g, lo=0, hi=D):
        return jnp.concatenate([head_weight(w, g, j, lo, hi) for j in range(A_GROUP)], axis=1)

    def dense(x, first, w, emit, side=()):
        def quadrant(i, j):
            return x[_rows(first + i * (ROWS // 2), ROWS // 2), j * D // 2:(j + 1) * D // 2]

        sums = _left_sums(quadrant)
        left = lambda n: sums[n] if n in sums else quadrant(n - 3, n - 3)
        per = ROWS // 16
        slots = (D // pair * 7 - 1) * per
        queue = [(j * slots // len(side), job) for j, job in enumerate(side)]
        seen = [0]

        def each(y):
            seen[0] += per
            while queue and queue[0][0] < seen[0]:
                at, job = queue.pop(0)
                r = at % per * 8
                job(pltpu.bitcast(y[r:r + 8, :LANES], I32) & zeros[...])

        for c in range(0, D, pair):
            emit(slice(c, c + pair), _strassen(left, lambda i, j: _bf16(
                w[i * D // 4:(i + 1) * D // 4, c + j * LANES:c + (j + 1) * LANES]), each))

    def project_b(wq_raw, wk_raw, wv_raw, bq_raw, bk_raw, bv_raw, wob_raw, bk, bvq, xb):
        xb_copy = chunked_copy(xb_hbm, xb, n_rows)
        bq_copy = chunked_copy(wqkv_hbm.at[:, 0:D], bq_raw, n_rows)
        bk_copy = chunked_copy(wqkv_hbm.at[:, D:2 * D], bk_raw, n_rows)
        bv_copy = chunked_copy(wqkv_hbm.at[:, 2 * D:3 * D], bv_raw, n_rows)
        bo_copy = chunked_copy(wob_hbm, wob_raw, 1)
        a_copies = [
            chunked_copy(src, dst, 2 * n_rows)
            for src, dst in ((wq_hbm, wq_raw), (wk_hbm, wk_raw), (wv_hbm, wv_raw))
        ]

        def project_to(dst, w, i, side):
            def emit(cols, y):
                for t in range(2):
                    dst[cols.start // LANES + t, _rows(B_PAD + i * ROWS, ROWS, 8), :] = (
                        y[:, t * LANES:(t + 1) * LANES])

            dense(xb, i * ROWS, w, emit, side)

        def k_step(i, carry):
            xb_copy(i).wait()
            bv_copy(i).wait()
            bq_copy(i).wait()
            rows = D // n_rows
            project_to(kb, bk, i, [
                functools.partial(pack_b_cols, raw, dst, i * rows + r, 16)
                for raw, dst in ((bv_raw, bvq.at[0]), (bq_raw, bvq.at[1]))
                for r in range(0, rows, 16)])
            return carry

        def vq_step(i, carry):
            steps = 2 * n_rows
            for copy in a_copies:
                copy(i).wait()

            def rest_operands(_):
                per = n_seg // 2 // steps

                def quadrant(a, b):
                    return jnp.concatenate([
                        xa[_rows(((a * steps + i) * per + s) * seg + head, rest),
                           b * D // 2:(b + 1) * D // 2].astype(F32)
                        for s in range(per)], axis=0)

                terms = _left_sums(quadrant)
                terms[3] = quadrant(0, 0).astype(BF16)
                terms[4] = quadrant(1, 1).astype(BF16)
                n = per * rest // 2
                for j in range(1, 8):
                    xa_left[j - 1, _rows(i * n, n), :] = _words(terms[j])

            n = D // steps
            side = [functools.partial(pack_b_out, wob_raw, _rows(i * n, n), part)
                    for part in range(16)]
            side += [functools.partial(pack_a_heads, raw, dst, i * n + r, 4)
                     for raw, dst in ((wq_raw, wq), (wk_raw, wk), (wv_raw, wv))
                     for r in range(0, n, 4)]
            project_to(vqb.at[i // n_rows], bvq.at[i // n_rows], i % n_rows,
                       side + [rest_operands])
            return carry

        for i in range(n_rows):
            bk_copy(i).start()
        for i in range(n_rows):
            xb_copy(i).start()
            bv_copy(i).start()
            bq_copy(i).start()
        zeros[...] = jnp.zeros(zeros.shape, I32)
        for t in range(n_tiles):
            kb[t, 0:B_PAD, :] = jnp.zeros((B_PAD, LANES), F32)
        for i in range(n_rows):
            bk_copy(i).wait()
            rows = D // n_rows
            pack_b_cols(bk_raw, bk, i * rows, rows, jnp.zeros(zeros.shape, I32))
        bo_copy(0).start()
        xa_copy(0).start()
        mem_copy(0).start()
        for i in range(n_rows):
            for copy in a_copies:
                copy(i).start()
        lax.fori_loop(0, n_rows, k_step, 0)
        for i in range(n_rows, 2 * n_rows):
            for copy in a_copies:
                copy(i).start()
        ao_copy(0).start()
        bo_copy(0).wait()
        xa_copy(0).wait()
        lax.fori_loop(0, 2 * n_rows, vq_step, 0)

    head_raw = pltpu.VMEM((D, H, DH), BF16)
    square_raw = pltpu.VMEM((D, D), BF16)
    pl.run_scoped(
        project_b, head_raw, head_raw, head_raw, square_raw, square_raw, square_raw,
        square_raw, pltpu.VMEM((D // 2, D), U32), pltpu.VMEM((2, D // 2, D), U32),
        pltpu.VMEM((S, D), BF16))

    def window_attention(r0, near_start):
        scale = (D // B_HEADS) ** -0.5
        lane = lax.broadcasted_iota(I32, (8, LANES), 1)
        row = lax.broadcasted_iota(I32, (8, LANES), 0)
        taps = [pl.ds(B_PAD + r0 - B_DIL * w, 8) for w in range(B_TAPS)]
        qs = [qb[t, taps[0], :] for t in range(n_tiles)]
        sums = []
        for tap in taps:
            x = qs[0] * kb[0, tap, :]
            for t in range(1, n_tiles):
                x = x + qs[t] * kb[t, tap, :]
            sums.append(x)
        for k in (1, 2):
            sums = [x + jnp.where((lane & k) != 0, pltpu.roll(x, k, 1),
                                  pltpu.roll(x, LANES - k, 1)) for x in sums]
        logits = [x * scale for x in sums]
        if near_start:
            logits = [jnp.where(row + r0 >= B_DIL * w, x, NEG) for w, x in enumerate(logits)]
        top = functools.reduce(jnp.maximum, logits)
        e = [jnp.exp(x - top) for x in logits]
        inv = 1.0 / functools.reduce(jnp.add, e)
        p = [x * inv for x in e]
        tiles = []
        for t in range(n_tiles):
            o = p[0] * vb[t, taps[0], :]
            for w in range(1, B_TAPS):
                o = o + p[w] * vb[t, taps[w], :]
            tiles.append(o)
        return jnp.concatenate(tiles, axis=1)

    def finish(rest_qkv, rest_acc, u, oa, staged):
        def rest_step(g, carry):
            rows = S // n_groups
            base = pl.multiple_of(g * rows, rows)
            pieces = rows // 8
            products = 3 * (A_GROUP * DH // pair) * 7
            seen = [0]
            done = []

            def each(_):
                seen[0] += 1
                while len(done) < min(pieces, (pieces + 2) * seen[0] // (products - 4)):
                    r = 8 * len(done)
                    done.append(window_attention(base + r, r < B_PAD))
                    if r % 16:
                        u[pl.ds(base + (n_rest * ROWS + r - 8), 16), :] = jnp.concatenate(
                            done[-2:], axis=0).astype(BF16)

            for m, w in enumerate((wq, wk, wv)):
                for c in range(0, A_GROUP * DH, pair):
                    rest_qkv[m, g, :, c:c + pair] = _strassen(
                        lambda n: _bf16(xa_left[n - 1]),
                        lambda i, j: head_weight(
                            w, g, c // DH + j, i * D // 2, (i + 1) * D // 2),
                        each)
            n = H * DH // n_groups
            wo[_rows(g * (n // 2), n // 2), :] = _words(woa_raw[_rows(g * n, n), :])
            n = ROWS // n_groups
            rest_acc[_rows(g * n, n), :] = jnp.zeros((n, D), F32)
            return carry

        def segment(s, memory):
            scale = DH ** -0.5
            row = lax.broadcasted_iota(I32, (L, L), 0)
            col = lax.broadcasted_iota(I32, (L, L), 1)
            mask = (row < M) | (row >= col)
            tokens = xa[_rows(s * seg, seg), :].astype(F32)
            h = jnp.concatenate([memory, tokens[:head]], axis=0).astype(BF16)
            heads = [slice(j * DH, (j + 1) * DH) for j in range(A_GROUP)]

            def with_rest(m, g, y):
                return jnp.concatenate([y, rest_qkv[m, g, _rows(s * rest, rest), :]], axis=0)

            def scores(q, k):
                return [_dot_nt(q[:, c], k[:, c]) for c in heads]

            def attend(g, sc, v):
                out = []
                for x, c in zip(sc, heads):
                    x = jnp.where(mask, x * scale, NEG)
                    e = jnp.exp(x - jnp.max(x, axis=-1, keepdims=True))
                    p = e / jnp.sum(e, axis=-1, keepdims=True)
                    o = _dot(p, v[:, c]).astype(BF16)
                    at = g * A_GROUP * DH + c.start
                    u[_rows(at // D * ROWS + s * rest, rest), at % D:at % D + DH] = o[A_PASS:]
                    out.append(o[:A_PASS])
                return out

            early = [_dot(h[:, :D // 2], group_weight(w, 0, 0, D // 2)) for w in (wq, wk, wv)]
            q, k, v = (
                with_rest(m, 0, _dot(h[:, D // 2:], group_weight(w, 0, D // 2, D)) + early[m])
                for m, w in enumerate((wq, wk, wv)))
            o = []
            for g in range(1, n_groups):
                q_next = with_rest(0, g, _dot(h, group_weight(wq, g)))
                sc = scores(q, k)
                k_next = with_rest(1, g, _dot(h, group_weight(wk, g)))
                v_next = with_rest(2, g, _dot(h, group_weight(wv, g)))
                o += attend(g - 1, sc, v)
                q, k, v = q_next, k_next, v_next
            sc = scores(q, k)
            split = H // 2
            y = _dot(jnp.concatenate(o[:split], axis=1), _bf16(wo[:split * DH // 2, :]))
            o += attend(n_groups - 1, sc, v)
            y = _dot(jnp.concatenate(o[split:], axis=1),
                     _bf16(wo[split * DH // 2:H * DH // 2, :])) + y
            oa[s] = y[M:].astype(BF16)
            return y[:M]

        def a_step(i, carry):
            memory = mem[...]
            for j in range(A_UNROLL):
                memory = segment(i * A_UNROLL + j, memory)
            mem[...] = memory
            for j in range(A_UNROLL):
                s = i * A_UNROLL + j
                pltpu.make_async_copy(
                    oa.at[s], out_hbm.at[_rows(s * seg, head, seg), 0:D], oa_sem).start()
            return carry

        def out_step(i, carry):
            block = jnp.maximum(i - (n_rest - 1), 0)
            rows = _rows(block * ROWS, ROWS)

            def emit(cols, y):
                y = y + rest_acc[:, cols]
                rest_acc[:, cols] = jnp.where(i < n_rest - 1, y, 0.0)
                staged[rows, cols] = y.astype(BF16)

            dense(u, i * ROWS, wo.at[_rows(jnp.minimum(i, n_rest) * (D // 2), D // 2)], emit)

            @pl.when(i == n_rest - 1)
            def _():
                @pl.loop(0, n_seg)
                def _(s):
                    pltpu.make_async_copy(
                        staged.at[_rows(s * rest, rest)],
                        out_hbm.at[_rows(s * seg + head, rest), 0:D], rest_sem).start()

            @pl.when(i >= n_rest)
            def _():
                pltpu.make_async_copy(
                    staged.at[rows],
                    out_hbm.at[_rows((block - 1) * ROWS, ROWS), D:2 * D], ob_sem).start()

            return carry

        for t in range(n_tiles):
            vb[t, 0:B_PAD, :] = jnp.broadcast_to(vb[t, B_PAD:B_PAD + 1, :], (B_PAD, LANES))
        ao_copy(0).wait()
        mem_copy(0).wait()
        mem[...] = mem_raw[...].astype(F32)
        lax.fori_loop(0, n_groups, rest_step, 0)
        lax.fori_loop(0, n_seg // A_UNROLL, a_step, 0)
        lax.fori_loop(0, n_rest + n_rows, out_step, 0)
        pltpu.make_async_copy(oa, oa, oa_sem).wait()
        first = staged.at[0:ROWS]
        pltpu.make_async_copy(first, first, rest_sem).wait()
        others = staged.at[ROWS:]
        pltpu.make_async_copy(others, others, ob_sem).wait()

    pl.run_scoped(
        finish,
        pltpu.VMEM((3, n_groups, ROWS, A_GROUP * DH), F32),
        pltpu.VMEM((ROWS, D), F32),
        pltpu.VMEM((n_rest * ROWS + S, D), BF16),
        pltpu.VMEM((n_seg, head, D), BF16),
        pltpu.VMEM((ROWS + S, D), BF16),
    )


@functools.partial(jax.jit, static_argnames=("A_seg_len",))
def pallas_concat_heads__memory_aug_recurrent_mem_tr__sliding_local_dilated__prompt_kernel(
    A_x: jax.Array,
    A_mem0: jax.Array,
    A_Wq: jax.Array,
    A_Wk: jax.Array,
    A_Wv: jax.Array,
    A_Wo: jax.Array,
    A_seg_len: int,
    B_x: jax.Array,
    B_wqkv: jax.Array,
    B_wo: jax.Array,
):
    batch, S, D = A_x.shape
    _, H, DH = A_Wq.shape
    M = A_mem0.shape[1]
    seg = int(A_seg_len)
    assert batch == 1 and B_x.shape == A_x.shape
    assert DH == LANES and D == 8 * LANES and D // B_HEADS == 32
    assert S % (seg * A_UNROLL) == 0 and S % ROWS == 0
    assert S // seg * (M + seg - A_PASS) == ROWS

    head_words = pltpu.VMEM(((H + 1) * (D // 2 + SKEW), DH), U32)

    out = pl.pallas_call(
        functools.partial(_kernel, seg=seg),
        out_shape=jax.ShapeDtypeStruct((S, 2 * D), BF16),
        in_specs=[pl.BlockSpec(memory_space=pl.ANY)] * 9,
        out_specs=pl.BlockSpec(memory_space=pl.ANY),
        scratch_shapes=[
            head_words, head_words, head_words,
            pltpu.VMEM(((H * DH + D) // 2, D), U32),
            pltpu.VMEM((H * DH, D), BF16),
            pltpu.VMEM((S, D), BF16),
            pltpu.VMEM((M, D), BF16),
            pltpu.VMEM((M, D), F32),
            pltpu.VMEM((7, ROWS // 4, D // 2), U32),
            pltpu.VMEM((D // LANES, B_PAD + S, LANES), F32),
            pltpu.VMEM((2, D // LANES, B_PAD + S, LANES), F32),
            pltpu.VMEM((8, LANES), I32),
            pltpu.SemaphoreType.DMA((10 * (S // ROWS) + 7,)),
        ],
        compiler_params=pltpu.CompilerParams(vmem_limit_bytes=126 * 1024 * 1024),
        name="concat_heads",
    )(
        A_x.reshape(S, D), A_mem0.reshape(M, D), A_Wq, A_Wk, A_Wv,
        A_Wo.reshape(H * DH, D), B_x.reshape(S, D), B_wqkv, B_wo,
    )
    return out.reshape(batch, S, 2 * D)
```

```python
import functools

import jax
import jax.numpy as jnp
from jax import lax
import jax.experimental.pallas as pl
import jax.experimental.pallas.tpu as pltpu

LANES = 128
NEG = -1000000000.0

B_HEADS = 32
B_TAPS = 8
B_DIL = 2
B_PAD = 16

A_GROUP = 4
A_UNROLL = 2
A_PASS = 32
ROWS = 512
SKEW = 8

F32 = jnp.float32
BF16 = jnp.bfloat16
U32 = jnp.uint32
I32 = jnp.int32


def _dot(a, b):
    return jnp.dot(a, b, preferred_element_type=F32)


def _dot_nt(a, b):
    return lax.dot_general(a, b, (((1,), (1,)), ((), ())), preferred_element_type=F32)


def _bf16(words):
    return pltpu.bitcast(words, BF16)


def _words(halves):
    return pltpu.bitcast(halves, U32)


def _rows(start, size, align=None):
    if not isinstance(start, int):
        start = pl.multiple_of(start, size if align is None else align)
    return pl.ds(start, size)


def _add(a, b):
    return (a.astype(F32) + b.astype(F32)).astype(BF16)


def _sub(a, b):
    return (a.astype(F32) - b.astype(F32)).astype(BF16)


def _left_sums(a):
    a11, a12, a21, a22 = a(0, 0), a(0, 1), a(1, 0), a(1, 1)
    return {1: _add(a11, a22), 2: _add(a21, a22), 5: _add(a11, a12),
            6: _sub(a21, a11), 7: _sub(a12, a22)}


def _strassen(left, b, each):
    def product(n, right):
        y = _dot(left(n), right)
        each(y)
        return y

    m5 = product(5, b(1, 1))
    m3 = product(3, _sub(b(0, 1), b(1, 1)))
    c12 = m3 + m5
    c22 = product(6, _add(b(0, 0), b(0, 1))) + m3
    m2 = product(2, b(0, 0))
    c22 = c22 - m2
    c11 = product(7, _add(b(1, 0), b(1, 1))) - m5
    m4 = product(4, _sub(b(1, 0), b(0, 0)))
    c11 = m4 + c11
    c21 = m4 + m2
    m1 = product(1, _add(b(0, 0), b(1, 1)))
    c11 = m1 + c11
    c22 = m1 + c22
    return jnp.concatenate(
        [jnp.concatenate([c11, c12], axis=1), jnp.concatenate([c21, c22], axis=1)], axis=0)


def _swap_blocks(xs, axis, unit, zero):
    n = len(xs)
    size = xs[0].shape[axis]
    pos = ((lax.broadcasted_iota(I32, zero.shape, axis) | zero) // unit) % n
    pos = jnp.tile(pos, (xs[0].shape[0] // zero.shape[0], xs[0].shape[1] // zero.shape[1]))
    xs = [pltpu.roll(x, t * unit, axis) if t else x for t, x in enumerate(xs)]
    out = []
    for j in range(n):
        y = xs[0]
        for t in range(1, n):
            y = jnp.where(pos == (j + t) % n, xs[t], y)
        out.append(y)
    return [pltpu.roll(y, size - j * unit, axis) if j else y for j, y in enumerate(out)]


def _kernel(
    xa_hbm, mem_hbm, wq_hbm, wk_hbm, wv_hbm, woa_hbm, xb_hbm, wqkv_hbm, wob_hbm,
    out_hbm,
    wq, wk, wv, wo, woa_raw, xa, mem_raw, mem, xa_left, kb, vqb, zeros, sems,
    *, seg,
):
    S, D = xa.shape
    _, H, DH = wq_hbm.shape
    M = mem.shape[0]
    L = M + seg
    n_seg = S // seg
    head = A_PASS - M
    rest = seg - head
    pitch = D // 2 + SKEW
    n_tiles = D // LANES
    n_rows = S // ROWS
    n_groups = H // A_GROUP
    n_rest = H * DH // D
    pair = 2 * LANES
    vb, qb = vqb.at[0], vqb.at[1]
    woa = wo.at[D // 2:]

    sem_ids = iter(range(sems.shape[0]))

    def chunked_copy(src, dst, n):
        rows = src.shape[0] // n
        base = [next(sem_ids) for _ in range(n)][0]
        return lambda i: pltpu.make_async_copy(
            src.at[_rows(i * rows, rows)], dst.at[_rows(i * rows, rows)], sems.at[base + i])

    ao_copy = chunked_copy(woa_hbm, woa_raw, 1)
    xa_copy = chunked_copy(xa_hbm, xa, 1)
    mem_copy = chunked_copy(mem_hbm, mem_raw, 1)
    oa_sem = sems.at[next(sem_ids)]
    ob_sem = sems.at[next(sem_ids)]
    rest_sem = sems.at[next(sem_ids)]

    def pack_b_cols(raw, dst, first, rows, zero):
        xs = [_words(raw[_rows(first, rows), t * LANES:(t + 1) * LANES])
              for t in range(n_tiles)]
        for j, x in enumerate(_swap_blocks(xs, 1, 4, zero)):
            dst[_rows(first // 2, rows // 2), j * LANES:(j + 1) * LANES] = x

    def pack_b_out(raw, cols, part, zero):
        g, th, jh = part // 4, part // 2 % 2, part % 2
        xs = [_words(raw[pl.ds((4 * th + t) * 128 + g * 32 + jh * 16, 16), cols])
              for t in range(4)]
        for j, x in enumerate(_swap_blocks(xs, 0, 2, zero)):
            wo[pl.ds((4 * jh + j) * 64 + g * 16 + th * 8, 8), cols] = x

    def pack_a_heads(raw, dst, first, rows, zero):
        half = jnp.tile((zero | 16).astype(U32), (H // 16, 1))
        for r in range(rows // 2):
            at = first // 2 + r
            a = _words(raw[2 * at])
            b = _words(raw[2 * at + 1])
            dst[pl.ds(at, H // 2, stride=pitch), :] = (a & 0xFFFF) | (b << half)
            dst[pl.ds(H // 2 * pitch + at, H // 2, stride=pitch), :] = (a >> half) | (
                b & jnp.uint32(0xFFFF0000))

    def head_weight(w, g, j, lo, hi):
        first = g * (A_GROUP * pitch) + j * pitch + lo // 2
        return _bf16(w[_rows(first, (hi - lo) // 2, 8), :])

    def group_weight(w, g, lo=0, hi=D):
        return jnp.concatenate([head_weight(w, g, j, lo, hi) for j in range(A_GROUP)], axis=1)

    def dense(x, first, w, emit, side=()):
        def quadrant(i, j):
            return x[_rows(first + i * (ROWS // 2), ROWS // 2), j * D // 2:(j + 1) * D // 2]

        sums = _left_sums(quadrant)
        left = lambda n: sums[n] if n in sums else quadrant(n - 3, n - 3)
        per = ROWS // 16
        slots = (D // pair * 7 - 1) * per
        queue = [(j * slots // len(side), job) for j, job in enumerate(side)]
        seen = [0]

        def each(y):
            seen[0] += per
            while queue and queue[0][0] < seen[0]:
                at, job = queue.pop(0)
                r = at % per * 8
                job(pltpu.bitcast(y[r:r + 8, :LANES], I32) & zeros[...])

        for c in range(0, D, pair):
            emit(slice(c, c + pair), _strassen(left, lambda i, j: _bf16(
                w[i * D // 4:(i + 1) * D // 4, c + j * LANES:c + (j + 1) * LANES]), each))

    def project_b(wq_raw, wk_raw, wv_raw, bq_raw, bk_raw, bv_raw, wob_raw, bk, bvq, xb):
        xb_copy = chunked_copy(xb_hbm, xb, n_rows)
        bq_copy = chunked_copy(wqkv_hbm.at[:, 0:D], bq_raw, n_rows)
        bk_copy = chunked_copy(wqkv_hbm.at[:, D:2 * D], bk_raw, n_rows)
        bv_copy = chunked_copy(wqkv_hbm.at[:, 2 * D:3 * D], bv_raw, n_rows)
        bo_copy = chunked_copy(wob_hbm, wob_raw, 1)
        a_copies = [
            chunked_copy(src, dst, 2 * n_rows)
            for src, dst in ((wq_hbm, wq_raw), (wk_hbm, wk_raw), (wv_hbm, wv_raw))
        ]

        def project_to(dst, w, i, side):
            def emit(cols, y):
                for t in range(2):
                    dst[cols.start // LANES + t, _rows(B_PAD + i * ROWS, ROWS, 8), :] = (
                        y[:, t * LANES:(t + 1) * LANES])

            dense(xb, i * ROWS, w, emit, side)

        def k_step(i, carry):
            xb_copy(i).wait()
            bv_copy(i).wait()
            bq_copy(i).wait()
            rows = D // n_rows
            project_to(kb, bk, i, [
                functools.partial(pack_b_cols, raw, dst, i * rows + r, 16)
                for raw, dst in ((bv_raw, bvq.at[0]), (bq_raw, bvq.at[1]))
                for r in range(0, rows, 16)])
            return carry

        def vq_step(i, carry):
            steps = 2 * n_rows
            for copy in a_copies:
                copy(i).wait()

            def rest_operands(_):
                per = n_seg // 2 // steps

                def quadrant(a, b):
                    return jnp.concatenate([
                        xa[_rows(((a * steps + i) * per + s) * seg + head, rest),
                           b * D // 2:(b + 1) * D // 2].astype(F32)
                        for s in range(per)], axis=0)

                terms = _left_sums(quadrant)
                terms[3] = quadrant(0, 0).astype(BF16)
                terms[4] = quadrant(1, 1).astype(BF16)
                n = per * rest // 2
                for j in range(1, 8):
                    xa_left[j - 1, _rows(i * n, n), :] = _words(terms[j])

            n = D // steps
            side = [functools.partial(pack_b_out, wob_raw, _rows(i * n, n), part)
                    for part in range(16)]
            side += [functools.partial(pack_a_heads, raw, dst, i * n + r, 4)
                     for raw, dst in ((wq_raw, wq), (wk_raw, wk), (wv_raw, wv))
                     for r in range(0, n, 4)]
            project_to(vqb.at[i // n_rows], bvq.at[i // n_rows], i % n_rows,
                       side + [rest_operands])
            return carry

        for i in range(n_rows):
            bk_copy(i).start()
        for i in range(n_rows):
            xb_copy(i).start()
            bv_copy(i).start()
            bq_copy(i).start()
        zeros[...] = jnp.zeros(zeros.shape, I32)
        for t in range(n_tiles):
            kb[t, 0:B_PAD, :] = jnp.zeros((B_PAD, LANES), F32)
        for i in range(n_rows):
            bk_copy(i).wait()
            rows = D // n_rows
            pack_b_cols(bk_raw, bk, i * rows, rows, jnp.zeros(zeros.shape, I32))
        bo_copy(0).start()
        xa_copy(0).start()
        mem_copy(0).start()
        for i in range(n_rows):
            for copy in a_copies:
                copy(i).start()
        lax.fori_loop(0, n_rows, k_step, 0)
        for i in range(n_rows, 2 * n_rows):
            for copy in a_copies:
                copy(i).start()
        ao_copy(0).start()
        bo_copy(0).wait()
        xa_copy(0).wait()
        lax.fori_loop(0, 2 * n_rows, vq_step, 0)

    head_raw = pltpu.VMEM((D, H, DH), BF16)
    square_raw = pltpu.VMEM((D, D), BF16)
    pl.run_scoped(
        project_b, head_raw, head_raw, head_raw, square_raw, square_raw, square_raw,
        square_raw, pltpu.VMEM((D // 2, D), U32), pltpu.VMEM((2, D // 2, D), U32),
        pltpu.VMEM((S, D), BF16))

    def window_attention(r0, near_start):
        scale = (D // B_HEADS) ** -0.5
        lane = lax.broadcasted_iota(I32, (8, LANES), 1)
        row = lax.broadcasted_iota(I32, (8, LANES), 0)
        taps = [pl.ds(B_PAD + r0 - B_DIL * w, 8) for w in range(B_TAPS)]
        qs = [qb[t, taps[0], :] for t in range(n_tiles)]
        sums = []
        for tap in taps:
            x = qs[0] * kb[0, tap, :]
            for t in range(1, n_tiles):
                x = x + qs[t] * kb[t, tap, :]
            sums.append(x)
        for k in (1, 2):
            sums = [x + jnp.where((lane & k) != 0, pltpu.roll(x, k, 1),
                                  pltpu.roll(x, LANES - k, 1)) for x in sums]
        logits = [x * scale for x in sums]
        if near_start:
            logits = [jnp.where(row + r0 >= B_DIL * w, x, NEG) for w, x in enumerate(logits)]
        top = functools.reduce(jnp.maximum, logits)
        e = [jnp.exp(x - top) for x in logits]
        inv = 1.0 / functools.reduce(jnp.add, e)
        p = [x * inv for x in e]
        tiles = []
        for t in range(n_tiles):
            o = p[0] * vb[t, taps[0], :]
            for w in range(1, B_TAPS):
                o = o + p[w] * vb[t, taps[w], :]
            tiles.append(o)
        return jnp.concatenate(tiles, axis=1)

    def finish(rest_qkv, rest_acc, u, oa, staged):
        def rest_step(g, carry):
            rows = S // n_groups
            base = pl.multiple_of(g * rows, rows)
            pieces = rows // 8
            products = 3 * (A_GROUP * DH // pair) * 7
            seen = [0]
            done = []

            def each(_):
                seen[0] += 1
                while len(done) < min(pieces, (pieces + 2) * seen[0] // (products - 4)):
                    r = 8 * len(done)
                    done.append(window_attention(base + r, r < B_PAD))
                    if r % 16:
                        u[pl.ds(base + (r - 8), 16), :] = jnp.concatenate(
                            done[-2:], axis=0).astype(BF16)

            for m, w in enumerate((wq, wk, wv)):
                for c in range(0, A_GROUP * DH, pair):
                    rest_qkv[m, g, :, c:c + pair] = _strassen(
                        lambda n: _bf16(xa_left[n - 1]),
                        lambda i, j: head_weight(
                            w, g, c // DH + j, i * D // 2, (i + 1) * D // 2),
                        each)
            for j in range(A_GROUP):
                slot = g * A_GROUP + j
                source = slot % (H // 2) * 2 + slot // (H // 2)
                woa[_rows(slot * (DH // 2), DH // 2), :] = _words(
                    woa_raw[_rows(source * DH, DH), :])
            n = ROWS // n_groups
            rest_acc[_rows(g * n, n), :] = jnp.zeros((n, D), F32)
            return carry

        def segment(s, memory):
            scale = DH ** -0.5
            row = lax.broadcasted_iota(I32, (L, L), 0)
            col = lax.broadcasted_iota(I32, (L, L), 1)
            mask = (row < M) | (row >= col)
            tokens = xa[_rows(s * seg, seg), :].astype(F32)
            h = jnp.concatenate([memory, tokens[:head]], axis=0).astype(BF16)
            heads = [slice(j * DH, (j + 1) * DH) for j in range(A_GROUP)]

            def with_rest(m, g, y):
                return jnp.concatenate([y, rest_qkv[m, g, _rows(s * rest, rest), :]], axis=0)

            def scores(q, k):
                return [_dot_nt(q[:, c], k[:, c]) for c in heads]

            def attend(g, sc, v):
                out = []
                for x, c in zip(sc, heads):
                    x = jnp.where(mask, x * scale, NEG)
                    e = jnp.exp(x - jnp.max(x, axis=-1, keepdims=True))
                    p = e / jnp.sum(e, axis=-1, keepdims=True)
                    o = _dot(p, v[:, c]).astype(BF16)
                    at = g * A_GROUP * DH + c.start
                    u[_rows(S + at // D * ROWS + s * rest, rest), at % D:at % D + DH] = (
                        o[A_PASS:])
                    out.append(o[:A_PASS])
                return out

            early = [_dot(h[:, :D // 2], group_weight(w, 0, 0, D // 2)) for w in (wq, wk, wv)]
            q, k, v = (
                with_rest(m, 0, _dot(h[:, D // 2:], group_weight(w, 0, D // 2, D)) + early[m])
                for m, w in enumerate((wq, wk, wv)))
            o = []
            for g in range(1, n_groups):
                q_next = with_rest(0, g, _dot(h, group_weight(wq, g)))
                sc = scores(q, k)
                k_next = with_rest(1, g, _dot(h, group_weight(wk, g)))
                v_next = with_rest(2, g, _dot(h, group_weight(wv, g)))
                o += attend(g - 1, sc, v)
                q, k, v = q_next, k_next, v_next
            sc = scores(q, k)
            split = H // 2
            y = _dot(jnp.concatenate(o[:split], axis=1), _bf16(woa[:split * DH // 2, :]))
            o += attend(n_groups - 1, sc, v)
            y = _dot(jnp.concatenate(o[split:], axis=1), _bf16(woa[split * DH // 2:, :])) + y
            oa[s] = y[M:].astype(BF16)
            return y[:M]

        def a_step(i, carry):
            memory = mem[...]
            for j in range(A_UNROLL):
                memory = segment(i * A_UNROLL + j, memory)
            mem[...] = memory
            for j in range(A_UNROLL):
                s = i * A_UNROLL + j
                pltpu.make_async_copy(
                    oa.at[s], out_hbm.at[_rows(s * seg, head, seg), 0:D], oa_sem).start()
            return carry

        def out_step(i, carry):
            rows = _rows(jnp.minimum(i, n_rows) * ROWS, ROWS)

            def emit(cols, y):
                y = y + rest_acc[:, cols]
                rest_acc[:, cols] = jnp.where(i >= n_rows, y, 0.0)
                staged[rows, cols] = y.astype(BF16)

            block = jnp.maximum(i - (n_rows - 1), 0)
            dense(u, i * ROWS, wo.at[_rows(block * (D // 2), D // 2)], emit)

            @pl.when(i < n_rows)
            def _():
                pltpu.make_async_copy(
                    staged.at[rows], out_hbm.at[rows, D:2 * D], ob_sem).start()

            return carry

        for t in range(n_tiles):
            vb[t, 0:B_PAD, :] = jnp.broadcast_to(vb[t, B_PAD:B_PAD + 1, :], (B_PAD, LANES))
        ao_copy(0).wait()
        mem_copy(0).wait()
        mem[...] = mem_raw[...].astype(F32)
        lax.fori_loop(0, n_groups, rest_step, 0)
        lax.fori_loop(0, n_seg // A_UNROLL, a_step, 0)
        lax.fori_loop(0, n_rest + n_rows, out_step, 0)

        @pl.loop(0, n_seg)
        def _(s):
            pltpu.make_async_copy(
                staged.at[_rows(S + s * rest, rest)],
                out_hbm.at[_rows(s * seg + head, rest), 0:D], rest_sem).start()

        pltpu.make_async_copy(oa, oa, oa_sem).wait()
        pltpu.make_async_copy(staged.at[:S], staged.at[:S], ob_sem).wait()
        pltpu.make_async_copy(staged.at[S:], staged.at[S:], rest_sem).wait()

    pl.run_scoped(
        finish,
        pltpu.VMEM((3, n_groups, ROWS, A_GROUP * DH), F32),
        pltpu.VMEM((ROWS, D), F32),
        pltpu.VMEM((n_rest * ROWS + S, D), BF16),
        pltpu.VMEM((n_seg, head, D), BF16),
        pltpu.VMEM((ROWS + S, D), BF16),
    )


@functools.partial(jax.jit, static_argnames=("A_seg_len",))
def pallas_concat_heads__memory_aug_recurrent_mem_tr__sliding_local_dilated__prompt_kernel(
    A_x: jax.Array,
    A_mem0: jax.Array,
    A_Wq: jax.Array,
    A_Wk: jax.Array,
    A_Wv: jax.Array,
    A_Wo: jax.Array,
    A_seg_len: int,
    B_x: jax.Array,
    B_wqkv: jax.Array,
    B_wo: jax.Array,
):
    batch, S, D = A_x.shape
    _, H, DH = A_Wq.shape
    M = A_mem0.shape[1]
    seg = int(A_seg_len)
    assert batch == 1 and B_x.shape == A_x.shape
    assert DH == LANES and D == 8 * LANES and D // B_HEADS == 32
    assert S % (seg * A_UNROLL) == 0 and S % ROWS == 0
    assert S // seg * (M + seg - A_PASS) == ROWS

    head_words = pltpu.VMEM((H * (D // 2 + SKEW) + D // 2 + 32, DH), U32)

    out = pl.pallas_call(
        functools.partial(_kernel, seg=seg),
        out_shape=jax.ShapeDtypeStruct((S, 2 * D), BF16),
        in_specs=[pl.BlockSpec(memory_space=pl.ANY)] * 9,
        out_specs=pl.BlockSpec(memory_space=pl.ANY),
        scratch_shapes=[
            head_words, head_words, head_words,
            pltpu.VMEM(((H * DH + D) // 2, D), U32),
            pltpu.VMEM((H * DH, D), BF16),
            pltpu.VMEM((S, D), BF16),
            pltpu.VMEM((M, D), BF16),
            pltpu.VMEM((M, D), F32),
            pltpu.VMEM((7, ROWS // 4, D // 2), U32),
            pltpu.VMEM((D // LANES, B_PAD + S, LANES), F32),
            pltpu.VMEM((2, D // LANES, B_PAD + S, LANES), F32),
            pltpu.VMEM((8, LANES), I32),
            pltpu.SemaphoreType.DMA((10 * (S // ROWS) + 7,)),
        ],
        compiler_params=pltpu.CompilerParams(vmem_limit_bytes=126 * 1024 * 1024),
        name="concat_heads",
    )(
        A_x.reshape(S, D), A_mem0.reshape(M, D), A_Wq, A_Wk, A_Wv,
        A_Wo.reshape(H * DH, D), B_x.reshape(S, D), B_wqkv, B_wo,
    )
    return out.reshape(batch, S, 2 * D)
```

```python
import functools

import jax
import jax.numpy as jnp
from jax import lax
import jax.experimental.pallas as pl
import jax.experimental.pallas.tpu as pltpu

LANES = 128
NEG = -1000000000.0

B_HEADS = 32
B_TAPS = 8
B_DIL = 2
B_PAD = 16

A_GROUP = 4
A_UNROLL = 2
A_PASS = 32
ROWS = 512
SKEW = 8

F32 = jnp.float32
BF16 = jnp.bfloat16
U32 = jnp.uint32
I32 = jnp.int32


def _dot(a, b):
    return jnp.dot(a, b, preferred_element_type=F32)


def _dot_nt(a, b):
    return lax.dot_general(a, b, (((1,), (1,)), ((), ())), preferred_element_type=F32)


def _bf16(words):
    return pltpu.bitcast(words, BF16)


def _words(halves):
    return pltpu.bitcast(halves, U32)


def _rows(start, size, align=None):
    if not isinstance(start, int):
        start = pl.multiple_of(start, size if align is None else align)
    return pl.ds(start, size)


def _add(a, b):
    return (a.astype(F32) + b.astype(F32)).astype(BF16)


def _sub(a, b):
    return (a.astype(F32) - b.astype(F32)).astype(BF16)


def _left_sums(a):
    a11, a12, a21, a22 = a(0, 0), a(0, 1), a(1, 0), a(1, 1)
    return {1: _add(a11, a22), 2: _add(a21, a22), 5: _add(a11, a12),
            6: _sub(a21, a11), 7: _sub(a12, a22)}


def _strassen(left, b, each):
    def product(n, right):
        y = _dot(left(n), right)
        each(y)
        return y

    m5 = product(5, b(1, 1))
    m3 = product(3, _sub(b(0, 1), b(1, 1)))
    c12 = m3 + m5
    c22 = product(6, _add(b(0, 0), b(0, 1))) + m3
    m2 = product(2, b(0, 0))
    c22 = c22 - m2
    c11 = product(7, _add(b(1, 0), b(1, 1))) - m5
    m4 = product(4, _sub(b(1, 0), b(0, 0)))
    c11 = m4 + c11
    c21 = m4 + m2
    m1 = product(1, _add(b(0, 0), b(1, 1)))
    c11 = m1 + c11
    c22 = m1 + c22
    return jnp.concatenate(
        [jnp.concatenate([c11, c12], axis=1), jnp.concatenate([c21, c22], axis=1)], axis=0)


def _swap_blocks(xs, axis, unit, zero):
    n = len(xs)
    size = xs[0].shape[axis]
    pos = ((lax.broadcasted_iota(I32, zero.shape, axis) | zero) // unit) % n
    pos = jnp.tile(pos, (xs[0].shape[0] // zero.shape[0], xs[0].shape[1] // zero.shape[1]))
    xs = [pltpu.roll(x, t * unit, axis) if t else x for t, x in enumerate(xs)]
    out = []
    for j in range(n):
        y = xs[0]
        for t in range(1, n):
            y = jnp.where(pos == (j + t) % n, xs[t], y)
        out.append(y)
    return [pltpu.roll(y, size - j * unit, axis) if j else y for j, y in enumerate(out)]


def _kernel(
    xa_hbm, mem_hbm, wq_hbm, wk_hbm, wv_hbm, woa_hbm, xb_hbm, wqkv_hbm, wob_hbm,
    out_hbm,
    wq, wk, wv, wo, woa_raw, xa, mem_raw, mem, xa_left, kb, vqb, zeros, sems,
    *, seg,
):
    S, D = xa.shape
    _, H, DH = wq_hbm.shape
    M = mem.shape[0]
    L = M + seg
    n_seg = S // seg
    head = A_PASS - M
    rest = seg - head
    pitch = D // 2 + SKEW
    n_tiles = D // LANES
    n_rows = S // ROWS
    n_groups = H // A_GROUP
    n_rest = H * DH // D
    pair = 2 * LANES
    vb, qb = vqb.at[0], vqb.at[1]
    woa = wo.at[D // 2:]

    sem_ids = iter(range(sems.shape[0]))

    def chunked_copy(src, dst, n):
        rows = src.shape[0] // n
        base = [next(sem_ids) for _ in range(n)][0]
        return lambda i: pltpu.make_async_copy(
            src.at[_rows(i * rows, rows)], dst.at[_rows(i * rows, rows)], sems.at[base + i])

    ao_copy = chunked_copy(woa_hbm, woa_raw, 1)
    xa_copy = chunked_copy(xa_hbm, xa, 4 * n_rows)
    mem_copy = chunked_copy(mem_hbm, mem_raw, 1)
    oa_sem = sems.at[next(sem_ids)]
    ob_sem = sems.at[next(sem_ids)]
    rest_sem = sems.at[next(sem_ids)]

    def pack_b_cols(raw, dst, first, rows, zero):
        xs = [_words(raw[_rows(first, rows), t * LANES:(t + 1) * LANES])
              for t in range(n_tiles)]
        for j, x in enumerate(_swap_blocks(xs, 1, 4, zero)):
            dst[_rows(first // 2, rows // 2), j * LANES:(j + 1) * LANES] = x

    def pack_b_out(raw, cols, part, zero):
        g, th, jh = part // 4, part // 2 % 2, part % 2
        xs = [_words(raw[pl.ds((4 * th + t) * 128 + g * 32 + jh * 16, 16), cols])
              for t in range(4)]
        for j, x in enumerate(_swap_blocks(xs, 0, 2, zero)):
            wo[pl.ds((4 * jh + j) * 64 + g * 16 + th * 8, 8), cols] = x

    def pack_a_heads(raw, dst, first, rows, zero):
        half = jnp.tile((zero | 16).astype(U32), (H // 16, 1))
        for r in range(rows // 2):
            at = first // 2 + r
            a = _words(raw[2 * at])
            b = _words(raw[2 * at + 1])
            dst[pl.ds(at, H // 2, stride=pitch), :] = (a & 0xFFFF) | (b << half)
            dst[pl.ds(H // 2 * pitch + at, H // 2, stride=pitch), :] = (a >> half) | (
                b & jnp.uint32(0xFFFF0000))

    def head_weight(w, g, j, lo, hi):
        first = g * (A_GROUP * pitch) + j * pitch + lo // 2
        return _bf16(w[_rows(first, (hi - lo) // 2, 8), :])

    def group_weight(w, g, lo=0, hi=D):
        return jnp.concatenate([head_weight(w, g, j, lo, hi) for j in range(A_GROUP)], axis=1)

    def dense(x, first, w, emit, side=()):
        def quadrant(i, j):
            return x[_rows(first + i * (ROWS // 2), ROWS // 2), j * D // 2:(j + 1) * D // 2]

        sums = _left_sums(quadrant)
        left = lambda n: sums[n] if n in sums else quadrant(n - 3, n - 3)
        per = ROWS // 16
        slots = (D // pair * 7 - 1) * per
        queue = [(j * slots // len(side), job) for j, job in enumerate(side)]
        seen = [0]

        def each(y):
            seen[0] += per
            while queue and queue[0][0] < seen[0]:
                at, job = queue.pop(0)
                r = at % per * 8
                job(pltpu.bitcast(y[r:r + 8, :LANES], I32) & zeros[...])

        for c in range(0, D, pair):
            emit(slice(c, c + pair), _strassen(left, lambda i, j: _bf16(
                w[i * D // 4:(i + 1) * D // 4, c + j * LANES:c + (j + 1) * LANES]), each))

    def project_b(wq_raw, wk_raw, wv_raw, bq_raw, bk_raw, bv_raw, wob_raw, bk, bvq, xb):
        xb_copy = chunked_copy(xb_hbm, xb, n_rows)
        bq_copy = chunked_copy(wqkv_hbm.at[:, 0:D], bq_raw, n_rows)
        bk_copy = chunked_copy(wqkv_hbm.at[:, D:2 * D], bk_raw, n_rows)
        bv_copy = chunked_copy(wqkv_hbm.at[:, 2 * D:3 * D], bv_raw, n_rows)
        bo_copy = chunked_copy(wob_hbm, wob_raw, 1)
        a_copies = [
            chunked_copy(src, dst, 2 * n_rows)
            for src, dst in ((wq_hbm, wq_raw), (wk_hbm, wk_raw), (wv_hbm, wv_raw))
        ] + [xa_copy, lambda i: xa_copy(2 * n_rows + i)]

        def project_to(dst, w, i, side):
            def emit(cols, y):
                for t in range(2):
                    dst[cols.start // LANES + t, _rows(B_PAD + i * ROWS, ROWS, 8), :] = (
                        y[:, t * LANES:(t + 1) * LANES])

            dense(xb, i * ROWS, w, emit, side)

        def k_step(i, carry):
            xb_copy(i).wait()
            bv_copy(i).wait()
            bq_copy(i).wait()
            rows = D // n_rows
            project_to(kb, bk, i, [
                functools.partial(pack_b_cols, raw, dst, i * rows + r, 16)
                for raw, dst in ((bv_raw, bvq.at[0]), (bq_raw, bvq.at[1]))
                for r in range(0, rows, 16)])
            return carry

        def vq_step(i, carry):
            steps = 2 * n_rows
            for copy in a_copies:
                copy(i).wait()

            def rest_operands(_):
                per = n_seg // 2 // steps

                def quadrant(a, b):
                    return jnp.concatenate([
                        xa[_rows(((a * steps + i) * per + s) * seg + head, rest),
                           b * D // 2:(b + 1) * D // 2].astype(F32)
                        for s in range(per)], axis=0)

                terms = _left_sums(quadrant)
                terms[3] = quadrant(0, 0).astype(BF16)
                terms[4] = quadrant(1, 1).astype(BF16)
                n = per * rest // 2
                for j in range(1, 8):
                    xa_left[j - 1, _rows(i * n, n), :] = _words(terms[j])

            n = D // steps
            side = [functools.partial(pack_b_out, wob_raw, _rows(i * n, n), part)
                    for part in range(16)]
            side += [functools.partial(pack_a_heads, raw, dst, i * n + r, 4)
                     for raw, dst in ((wq_raw, wq), (wk_raw, wk), (wv_raw, wv))
                     for r in range(0, n, 4)]
            project_to(vqb.at[i // n_rows], bvq.at[i // n_rows], i % n_rows,
                       side + [rest_operands])
            return carry

        for i in range(n_rows):
            bk_copy(i).start()
        for i in range(n_rows):
            xb_copy(i).start()
            bv_copy(i).start()
            bq_copy(i).start()
        zeros[...] = jnp.zeros(zeros.shape, I32)
        for t in range(n_tiles):
            kb[t, 0:B_PAD, :] = jnp.zeros((B_PAD, LANES), F32)
        for i in range(n_rows):
            bk_copy(i).wait()
            rows = D // n_rows
            pack_b_cols(bk_raw, bk, i * rows, rows, jnp.zeros(zeros.shape, I32))
        bo_copy(0).start()
        mem_copy(0).start()
        for i in range(n_rows):
            for copy in a_copies:
                copy(i).start()
        lax.fori_loop(0, n_rows, k_step, 0)
        for i in range(n_rows, 2 * n_rows):
            for copy in a_copies:
                copy(i).start()
        ao_copy(0).start()
        bo_copy(0).wait()
        lax.fori_loop(0, 2 * n_rows, vq_step, 0)

    head_raw = pltpu.VMEM((D, H, DH), BF16)
    square_raw = pltpu.VMEM((D, D), BF16)
    pl.run_scoped(
        project_b, head_raw, head_raw, head_raw, square_raw, square_raw, square_raw,
        square_raw, pltpu.VMEM((D // 2, D), U32), pltpu.VMEM((2, D // 2, D), U32),
        pltpu.VMEM((S, D), BF16))

    def window_attention(r0, near_start):
        scale = (D // B_HEADS) ** -0.5
        lane = lax.broadcasted_iota(I32, (8, LANES), 1)
        row = lax.broadcasted_iota(I32, (8, LANES), 0)
        taps = [pl.ds(B_PAD + r0 - B_DIL * w, 8) for w in range(B_TAPS)]
        qs = [qb[t, taps[0], :] for t in range(n_tiles)]
        sums = []
        for tap in taps:
            x = qs[0] * kb[0, tap, :]
            for t in range(1, n_tiles):
                x = x + qs[t] * kb[t, tap, :]
            sums.append(x)
        for k in (1, 2):
            sums = [x + jnp.where((lane & k) != 0, pltpu.roll(x, k, 1),
                                  pltpu.roll(x, LANES - k, 1)) for x in sums]
        logits = [x * scale for x in sums]
        if near_start:
            logits = [jnp.where(row + r0 >= B_DIL * w, x, NEG) for w, x in enumerate(logits)]
        top = functools.reduce(jnp.maximum, logits)
        e = [jnp.exp(x - top) for x in logits]
        inv = 1.0 / functools.reduce(jnp.add, e)
        p = [x * inv for x in e]
        tiles = []
        for t in range(n_tiles):
            o = p[0] * vb[t, taps[0], :]
            for w in range(1, B_TAPS):
                o = o + p[w] * vb[t, taps[w], :]
            tiles.append(o)
        return jnp.concatenate(tiles, axis=1)

    def finish(rest_qkv, rest_acc, u, oa, staged):
        def rest_step(g, carry):
            rows = S // n_groups
            base = pl.multiple_of(g * rows, rows)
            pieces = rows // 8
            products = 3 * (A_GROUP * DH // pair) * 7
            seen = [0]
            done = []

            def each(_):
                seen[0] += 1
                while len(done) < min(pieces, (pieces + 2) * seen[0] // (products - 4)):
                    r = 8 * len(done)
                    done.append(window_attention(base + r, r < B_PAD))
                    if r % 16:
                        u[pl.ds(base + (r - 8), 16), :] = jnp.concatenate(
                            done[-2:], axis=0).astype(BF16)

            for m, w in enumerate((wq, wk, wv)):
                for c in range(0, A_GROUP * DH, pair):
                    rest_qkv[m, g, :, c:c + pair] = _strassen(
                        lambda n: _bf16(xa_left[n - 1]),
                        lambda i, j: head_weight(
                            w, g, c // DH + j, i * D // 2, (i + 1) * D // 2),
                        each)
            for j in range(A_GROUP):
                slot = g * A_GROUP + j
                source = slot % (H // 2) * 2 + slot // (H // 2)
                woa[_rows(slot * (DH // 2), DH // 2), :] = _words(
                    woa_raw[_rows(source * DH, DH), :])
            n = ROWS // n_groups
            rest_acc[_rows(g * n, n), :] = jnp.zeros((n, D), F32)
            return carry

        def segment(s, memory):
            scale = DH ** -0.5
            row = lax.broadcasted_iota(I32, (L, L), 0)
            col = lax.broadcasted_iota(I32, (L, L), 1)
            mask = (row < M) | (row >= col)
            tokens = xa[_rows(s * seg, seg), :].astype(F32)
            h = jnp.concatenate([memory, tokens[:head]], axis=0).astype(BF16)
            heads = [slice(j * DH, (j + 1) * DH) for j in range(A_GROUP)]

            def with_rest(m, g, y):
                return jnp.concatenate([y, rest_qkv[m, g, _rows(s * rest, rest), :]], axis=0)

            def scores(q, k):
                return [_dot_nt(q[:, c], k[:, c]) for c in heads]

            def attend(g, sc, v):
                out = []
                for x, c in zip(sc, heads):
                    x = jnp.where(mask, x * scale, NEG)
                    e = jnp.exp(x - jnp.max(x, axis=-1, keepdims=True))
                    p = e / jnp.sum(e, axis=-1, keepdims=True)
                    o = _dot(p, v[:, c]).astype(BF16)
                    at = g * A_GROUP * DH + c.start
                    u[_rows(S + at // D * ROWS + s * rest, rest), at % D:at % D + DH] = (
                        o[A_PASS:])
                    out.append(o[:A_PASS])
                return out

            early = [_dot(h[:, :D // 2], group_weight(w, 0, 0, D // 2)) for w in (wq, wk, wv)]
            q, k, v = (
                with_rest(m, 0, _dot(h[:, D // 2:], group_weight(w, 0, D // 2, D)) + early[m])
                for m, w in enumerate((wq, wk, wv)))
            o = []
            for g in range(1, n_groups):
                q_next = with_rest(0, g, _dot(h, group_weight(wq, g)))
                sc = scores(q, k)
                k_next = with_rest(1, g, _dot(h, group_weight(wk, g)))
                v_next = with_rest(2, g, _dot(h, group_weight(wv, g)))
                o += attend(g - 1, sc, v)
                q, k, v = q_next, k_next, v_next
            sc = scores(q, k)
            split = H // 2
            y = _dot(jnp.concatenate(o[:split], axis=1), _bf16(woa[:split * DH // 2, :]))
            o += attend(n_groups - 1, sc, v)
            y = _dot(jnp.concatenate(o[split:], axis=1), _bf16(woa[split * DH // 2:, :])) + y
            oa[s] = y[M:].astype(BF16)
            return y[:M]

        def a_step(i, carry):
            memory = mem[...]
            for j in range(A_UNROLL):
                memory = segment(i * A_UNROLL + j, memory)
            mem[...] = memory
            for j in range(A_UNROLL):
                s = i * A_UNROLL + j
                pltpu.make_async_copy(
                    oa.at[s], out_hbm.at[_rows(s * seg, head, seg), 0:D], oa_sem).start()
            return carry

        def out_step(i, carry):
            rows = _rows(jnp.minimum(i, n_rows) * ROWS, ROWS)

            def emit(cols, y):
                y = y + rest_acc[:, cols]
                rest_acc[:, cols] = jnp.where(i >= n_rows, y, 0.0)
                staged[rows, cols] = y.astype(BF16)

            block = jnp.maximum(i - (n_rows - 1), 0)
            dense(u, i * ROWS, wo.at[_rows(block * (D // 2), D // 2)], emit)

            @pl.when(i < n_rows)
            def _():
                pltpu.make_async_copy(
                    staged.at[rows], out_hbm.at[rows, D:2 * D], ob_sem).start()

            return carry

        for t in range(n_tiles):
            vb[t, 0:B_PAD, :] = jnp.broadcast_to(vb[t, B_PAD:B_PAD + 1, :], (B_PAD, LANES))
        ao_copy(0).wait()
        mem_copy(0).wait()
        mem[...] = mem_raw[...].astype(F32)
        lax.fori_loop(0, n_groups, rest_step, 0)
        lax.fori_loop(0, n_seg // A_UNROLL, a_step, 0)
        lax.fori_loop(0, n_rest + n_rows, out_step, 0)

        @pl.loop(0, n_seg)
        def _(s):
            pltpu.make_async_copy(
                staged.at[_rows(S + s * rest, rest)],
                out_hbm.at[_rows(s * seg + head, rest), 0:D], rest_sem).start()

        pltpu.make_async_copy(oa, oa, oa_sem).wait()
        pltpu.make_async_copy(staged.at[:S], staged.at[:S], ob_sem).wait()
        pltpu.make_async_copy(staged.at[S:], staged.at[S:], rest_sem).wait()

    pl.run_scoped(
        finish,
        pltpu.VMEM((3, n_groups, ROWS, A_GROUP * DH), F32),
        pltpu.VMEM((ROWS, D), F32),
        pltpu.VMEM((n_rest * ROWS + S, D), BF16),
        pltpu.VMEM((n_seg, head, D), BF16),
        pltpu.VMEM((ROWS + S, D), BF16),
    )


@functools.partial(jax.jit, static_argnames=("A_seg_len",))
def pallas_concat_heads__memory_aug_recurrent_mem_tr__sliding_local_dilated__prompt_kernel(
    A_x: jax.Array,
    A_mem0: jax.Array,
    A_Wq: jax.Array,
    A_Wk: jax.Array,
    A_Wv: jax.Array,
    A_Wo: jax.Array,
    A_seg_len: int,
    B_x: jax.Array,
    B_wqkv: jax.Array,
    B_wo: jax.Array,
):
    batch, S, D = A_x.shape
    _, H, DH = A_Wq.shape
    M = A_mem0.shape[1]
    seg = int(A_seg_len)
    assert batch == 1 and B_x.shape == A_x.shape
    assert DH == LANES and D == 8 * LANES and D // B_HEADS == 32
    assert S % (seg * A_UNROLL) == 0 and S % ROWS == 0
    assert S // seg * (M + seg - A_PASS) == ROWS

    head_words = pltpu.VMEM((H * (D // 2 + SKEW) + D // 2 + 32, DH), U32)

    out = pl.pallas_call(
        functools.partial(_kernel, seg=seg),
        out_shape=jax.ShapeDtypeStruct((S, 2 * D), BF16),
        in_specs=[pl.BlockSpec(memory_space=pl.ANY)] * 9,
        out_specs=pl.BlockSpec(memory_space=pl.ANY),
        scratch_shapes=[
            head_words, head_words, head_words,
            pltpu.VMEM(((H * DH + D) // 2, D), U32),
            pltpu.VMEM((H * DH, D), BF16),
            pltpu.VMEM((S, D), BF16),
            pltpu.VMEM((M, D), BF16),
            pltpu.VMEM((M, D), F32),
            pltpu.VMEM((7, ROWS // 4, D // 2), U32),
            pltpu.VMEM((D // LANES, B_PAD + S, LANES), F32),
            pltpu.VMEM((2, D // LANES, B_PAD + S, LANES), F32),
            pltpu.VMEM((8, LANES), I32),
            pltpu.SemaphoreType.DMA((14 * (S // ROWS) + 6,)),
        ],
        compiler_params=pltpu.CompilerParams(vmem_limit_bytes=126 * 1024 * 1024),
        name="concat_heads",
    )(
        A_x.reshape(S, D), A_mem0.reshape(M, D), A_Wq, A_Wk, A_Wv,
        A_Wo.reshape(H * DH, D), B_x.reshape(S, D), B_wqkv, B_wo,
    )
    return out.reshape(batch, S, 2 * D)
```

```python
import functools

import jax
import jax.numpy as jnp
from jax import lax
import jax.experimental.pallas as pl
import jax.experimental.pallas.tpu as pltpu

LANES = 128
NEG = -1000000000.0

B_HEADS = 32
B_TAPS = 8
B_DIL = 2
B_PAD = 16

A_GROUP = 4
A_UNROLL = 2
A_PASS = 32
ROWS = 512
SKEW = 8

F32 = jnp.float32
BF16 = jnp.bfloat16
U32 = jnp.uint32
I32 = jnp.int32


def _dot(a, b):
    return jnp.dot(a, b, preferred_element_type=F32)


def _dot_nt(a, b):
    return lax.dot_general(a, b, (((1,), (1,)), ((), ())), preferred_element_type=F32)


def _bf16(words):
    return pltpu.bitcast(words, BF16)


def _words(halves):
    return pltpu.bitcast(halves, U32)


def _rows(start, size, align=None):
    if not isinstance(start, int):
        start = pl.multiple_of(start, size if align is None else align)
    return pl.ds(start, size)


def _add(a, b):
    return (a.astype(F32) + b.astype(F32)).astype(BF16)


def _sub(a, b):
    return (a.astype(F32) - b.astype(F32)).astype(BF16)


def _left_sums(a):
    a11, a12, a21, a22 = a(0, 0), a(0, 1), a(1, 0), a(1, 1)
    return {1: _add(a11, a22), 2: _add(a21, a22), 5: _add(a11, a12),
            6: _sub(a21, a11), 7: _sub(a12, a22)}


_PRODUCTS = {
    1: (lambda b: _add(b(0, 0), b(1, 1)), ((0, 1), (3, 1))),
    2: (lambda b: b(0, 0), ((2, 1), (3, -1))),
    3: (lambda b: _sub(b(0, 1), b(1, 1)), ((1, 1), (3, 1))),
    4: (lambda b: _sub(b(1, 0), b(0, 0)), ((0, 1), (2, 1))),
    5: (lambda b: b(1, 1), ((0, -1), (1, 1))),
    6: (lambda b: _add(b(0, 0), b(0, 1)), ((3, 1),)),
    7: (lambda b: _add(b(1, 0), b(1, 1)), ((0, 1),)),
}


def _strassen(left, b, each, order):
    c = [None] * 4
    signs = [1] * 4
    for n in order:
        right, uses = _PRODUCTS[n]
        y = _dot(left(n), right(b))
        each(y)
        for q, sign in uses:
            if c[q] is None:
                c[q], signs[q] = y, sign
            elif sign < 0:
                c[q] = c[q] - y
            else:
                c[q], signs[q] = (y + c[q] if signs[q] > 0 else y - c[q]), 1
    return jnp.concatenate(
        [jnp.concatenate(c[:2], axis=1), jnp.concatenate(c[2:], axis=1)], axis=0)


def _swap_blocks(xs, axis, unit, zero):
    n = len(xs)
    size = xs[0].shape[axis]
    pos = ((lax.broadcasted_iota(I32, zero.shape, axis) | zero) // unit) % n
    pos = jnp.tile(pos, (xs[0].shape[0] // zero.shape[0], xs[0].shape[1] // zero.shape[1]))
    xs = [pltpu.roll(x, t * unit, axis) if t else x for t, x in enumerate(xs)]
    out = []
    for j in range(n):
        y = xs[0]
        for t in range(1, n):
            y = jnp.where(pos == (j + t) % n, xs[t], y)
        out.append(y)
    return [pltpu.roll(y, size - j * unit, axis) if j else y for j, y in enumerate(out)]


def _kernel(
    xa_hbm, mem_hbm, wq_hbm, wk_hbm, wv_hbm, woa_hbm, xb_hbm, wqkv_hbm, wob_hbm,
    out_hbm,
    wq, wk, wv, wo, woa_raw, xa, mem_raw, mem, xa_left, kb, vqb, zeros, sems,
    *, seg,
):
    S, D = xa.shape
    _, H, DH = wq_hbm.shape
    M = mem.shape[0]
    L = M + seg
    n_seg = S // seg
    head = A_PASS - M
    rest = seg - head
    pitch = D // 2 + SKEW
    n_tiles = D // LANES
    n_rows = S // ROWS
    n_groups = H // A_GROUP
    n_rest = H * DH // D
    pair = 2 * LANES
    vb, qb = vqb.at[0], vqb.at[1]
    woa = wo.at[D // 2:]

    sem_ids = iter(range(sems.shape[0]))

    def chunked_copy(src, dst, n):
        rows = src.shape[0] // n
        base = [next(sem_ids) for _ in range(n)][0]
        return lambda i: pltpu.make_async_copy(
            src.at[_rows(i * rows, rows)], dst.at[_rows(i * rows, rows)], sems.at[base + i])

    ao_copy = chunked_copy(woa_hbm, woa_raw, 1)
    xa_copy = chunked_copy(xa_hbm, xa, 4 * n_rows)
    mem_copy = chunked_copy(mem_hbm, mem_raw, 1)
    oa_sem = sems.at[next(sem_ids)]
    ob_sem = sems.at[next(sem_ids)]
    rest_sem = sems.at[next(sem_ids)]

    def pack_b_cols(raw, dst, first, rows):
        xs = [_words(raw[_rows(first, rows), t * LANES:(t + 1) * LANES])
              for t in range(n_tiles)]
        for j, x in enumerate(_swap_blocks(xs, 1, 4, jnp.zeros((8, LANES), I32))):
            dst[_rows(first // 2, rows // 2), j * LANES:(j + 1) * LANES] = x

    def pack_b_out(raw, cols, part, zero):
        g, th, jh = part // 4, part // 2 % 2, part % 2
        xs = [_words(raw[pl.ds((4 * th + t) * 128 + g * 32 + jh * 16, 16), cols])
              for t in range(4)]
        for j, x in enumerate(_swap_blocks(xs, 0, 2, zero)):
            wo[pl.ds((4 * jh + j) * 64 + g * 16 + th * 8, 8), cols] = x

    def pack_a_heads(raw, dst, first, rows, zero):
        half = jnp.tile((zero | 16).astype(U32), (H // 16, 1))
        for r in range(rows // 2):
            at = first // 2 + r
            a = _words(raw[2 * at])
            b = _words(raw[2 * at + 1])
            dst[pl.ds(at, H // 2, stride=pitch), :] = (a & 0xFFFF) | (b << half)
            dst[pl.ds(H // 2 * pitch + at, H // 2, stride=pitch), :] = (a >> half) | (
                b & jnp.uint32(0xFFFF0000))

    def head_weight(w, g, j, lo, hi):
        first = g * (A_GROUP * pitch) + j * pitch + lo // 2
        return _bf16(w[_rows(first, (hi - lo) // 2, 8), :])

    def group_weight(w, g, lo=0, hi=D):
        return jnp.concatenate([head_weight(w, g, j, lo, hi) for j in range(A_GROUP)], axis=1)

    def quadrants(x, first):
        return lambda i, j: x[_rows(first + i * (ROWS // 2), ROWS // 2),
                              j * D // 2:(j + 1) * D // 2]

    def dense(a, sums, w, emit, order, side=()):
        per = ROWS // 16
        slots = (D // pair * 7 - 1) * per
        queue = [(j * slots // len(side), job) for j, job in enumerate(side)]
        seen = [0]

        def each(y):
            seen[0] += per
            while queue and queue[0][0] < seen[0]:
                at, job = queue.pop(0)
                r = at % per * 8
                job(pltpu.bitcast(y[r:r + 8, :LANES], I32) & zeros[...])

        for c in range(0, D, pair):
            emit(slice(c, c + pair), _strassen(
                lambda n: a(n - 3, n - 3) if n in (3, 4) else sums(n),
                lambda i, j: _bf16(
                    w[i * D // 4:(i + 1) * D // 4, c + j * LANES:c + (j + 1) * LANES]),
                each, order))

    def project_b(wq_raw, wk_raw, wv_raw, bq_raw, bk_raw, bv_raw, wob_raw, bk, bvq,
                  xb, xb_left):
        xb_copy = chunked_copy(xb_hbm, xb, n_rows)
        bq_copy = chunked_copy(wqkv_hbm.at[:, 0:D], bq_raw, n_rows)
        bk_copy = chunked_copy(wqkv_hbm.at[:, D:2 * D], bk_raw, n_rows)
        bv_copy = chunked_copy(wqkv_hbm.at[:, 2 * D:3 * D], bv_raw, n_rows)
        bo_copy = chunked_copy(wob_hbm, wob_raw, 1)
        a_copies = [
            chunked_copy(src, dst, 2 * n_rows)
            for src, dst in ((wq_hbm, wq_raw), (wk_hbm, wk_raw), (wv_hbm, wv_raw))
        ] + [xa_copy, lambda i: xa_copy(2 * n_rows + i)]

        def store_in(dst, i):
            def emit(cols, y):
                for t in range(2):
                    dst[cols.start // LANES + t, _rows(B_PAD + i * ROWS, ROWS, 8), :] = (
                        y[:, t * LANES:(t + 1) * LANES])

            return emit

        def k_step(i, carry):
            xb_copy(i).wait()
            bv_copy(i).wait()
            bq_copy(i).wait()
            a = quadrants(xb, i * ROWS)
            sums = _left_sums(a)
            for j, n in enumerate(sums):
                xb_left[i, j] = _words(sums[n])
            dense(a, sums.get, bk, store_in(kb, i), (6, 2, 3, 5, 1, 4, 7))
            rows = D // n_rows
            for raw, dst in ((bv_raw, bvq.at[0]), (bq_raw, bvq.at[1])):
                for r in range(0, rows, 16):
                    pack_b_cols(raw, dst, i * rows + r, 16)
            return carry

        def vq_step(i, carry):
            steps = 2 * n_rows
            for copy in a_copies:
                copy(i).wait()

            def rest_operands(_):
                per = n_seg // 2 // steps

                def quadrant(a, b):
                    return jnp.concatenate([
                        xa[_rows(((a * steps + i) * per + s) * seg + head, rest),
                           b * D // 2:(b + 1) * D // 2].astype(F32)
                        for s in range(per)], axis=0)

                terms = _left_sums(quadrant)
                terms[3] = quadrant(0, 0).astype(BF16)
                terms[4] = quadrant(1, 1).astype(BF16)
                n = per * rest // 2
                for j in range(1, 8):
                    xa_left[j - 1, _rows(i * n, n), :] = _words(terms[j])

            n = D // steps
            side = [functools.partial(pack_b_out, wob_raw, _rows(i * n, n), part)
                    for part in range(16)]
            side += [functools.partial(pack_a_heads, raw, dst, i * n + r, 4)
                     for raw, dst in ((wq_raw, wq), (wk_raw, wk), (wv_raw, wv))
                     for r in range(0, n, 4)]
            which, block = i // n_rows, i % n_rows
            dense(quadrants(xb, block * ROWS),
                  lambda n: _bf16(xb_left[block, (1, 2, 5, 6, 7).index(n)]),
                  bvq.at[which], store_in(vqb.at[which], block), (6, 2, 3, 1, 5, 7, 4),
                  side + [rest_operands])
            return carry

        for i in range(n_rows):
            bk_copy(i).start()
        for i in range(n_rows):
            xb_copy(i).start()
            bv_copy(i).start()
            bq_copy(i).start()
        zeros[...] = jnp.zeros(zeros.shape, I32)
        for t in range(n_tiles):
            kb[t, 0:B_PAD, :] = jnp.zeros((B_PAD, LANES), F32)
        for i in range(n_rows):
            bk_copy(i).wait()
            rows = D // n_rows
            pack_b_cols(bk_raw, bk, i * rows, rows)
        bo_copy(0).start()
        mem_copy(0).start()
        for i in range(n_rows):
            for copy in a_copies:
                copy(i).start()
        lax.fori_loop(0, n_rows, k_step, 0)
        for i in range(n_rows, 2 * n_rows):
            for copy in a_copies:
                copy(i).start()
        ao_copy(0).start()
        bo_copy(0).wait()
        lax.fori_loop(0, 2 * n_rows, vq_step, 0)

    head_raw = pltpu.VMEM((D, H, DH), BF16)
    square_raw = pltpu.VMEM((D, D), BF16)
    pl.run_scoped(
        project_b, head_raw, head_raw, head_raw, square_raw, square_raw, square_raw,
        square_raw, pltpu.VMEM((D // 2, D), U32), pltpu.VMEM((2, D // 2, D), U32),
        pltpu.VMEM((S, D), BF16), pltpu.VMEM((n_rows, 5, ROWS // 4, D // 2), U32))

    def window_attention(r0, near_start):
        scale = (D // B_HEADS) ** -0.5
        lane = lax.broadcasted_iota(I32, (8, LANES), 1)
        row = lax.broadcasted_iota(I32, (8, LANES), 0)
        taps = [pl.ds(B_PAD + r0 - B_DIL * w, 8) for w in range(B_TAPS)]
        qs = [qb[t, taps[0], :] for t in range(n_tiles)]
        sums = []
        for tap in taps:
            x = qs[0] * kb[0, tap, :]
            for t in range(1, n_tiles):
                x = x + qs[t] * kb[t, tap, :]
            sums.append(x)
        for k in (1, 2):
            sums = [x + jnp.where((lane & k) != 0, pltpu.roll(x, k, 1),
                                  pltpu.roll(x, LANES - k, 1)) for x in sums]
        logits = [x * scale for x in sums]
        if near_start:
            logits = [jnp.where(row + r0 >= B_DIL * w, x, NEG) for w, x in enumerate(logits)]
        top = functools.reduce(jnp.maximum, logits)
        e = [jnp.exp(x - top) for x in logits]
        inv = 1.0 / functools.reduce(jnp.add, e)
        p = [x * inv for x in e]
        tiles = []
        for t in range(n_tiles):
            o = p[0] * vb[t, taps[0], :]
            for w in range(1, B_TAPS):
                o = o + p[w] * vb[t, taps[w], :]
            tiles.append(o)
        return jnp.concatenate(tiles, axis=1)

    def finish(rest_qkv, rest_acc, u, oa, staged):
        def rest_step(g, carry):
            rows = S // n_groups
            base = pl.multiple_of(g * rows, rows)
            pieces = rows // 8
            products = 3 * (A_GROUP * DH // pair) * 7
            seen = [0]
            done = []

            def each(_):
                seen[0] += 1
                while len(done) < min(pieces, (pieces + 2) * seen[0] // (products - 4)):
                    r = 8 * len(done)
                    done.append(window_attention(base + r, r < B_PAD))
                    if r % 16:
                        u[pl.ds(base + (r - 8), 16), :] = jnp.concatenate(
                            done[-2:], axis=0).astype(BF16)

            for m, w in enumerate((wq, wk, wv)):
                for c in range(0, A_GROUP * DH, pair):
                    rest_qkv[m, g, :, c:c + pair] = _strassen(
                        lambda n: _bf16(xa_left[n - 1]),
                        lambda i, j: head_weight(
                            w, g, c // DH + j, i * D // 2, (i + 1) * D // 2),
                        each, (2, 6, 3, 7, 1, 4, 5))
            for j in range(A_GROUP):
                slot = g * A_GROUP + j
                source = slot % (H // 2) * 2 + slot // (H // 2)
                woa[_rows(slot * (DH // 2), DH // 2), :] = _words(
                    woa_raw[_rows(source * DH, DH), :])
            n = ROWS // n_groups
            rest_acc[_rows(g * n, n), :] = jnp.zeros((n, D), F32)
            return carry

        def segment(s, memory):
            scale = DH ** -0.5
            row = lax.broadcasted_iota(I32, (L, L), 0)
            col = lax.broadcasted_iota(I32, (L, L), 1)
            mask = (row < M) | (row >= col)
            tokens = xa[_rows(s * seg, seg), :].astype(F32)
            h = jnp.concatenate([memory, tokens[:head]], axis=0).astype(BF16)
            heads = [slice(j * DH, (j + 1) * DH) for j in range(A_GROUP)]

            def with_rest(m, g, y):
                return jnp.concatenate([y, rest_qkv[m, g, _rows(s * rest, rest), :]], axis=0)

            def scores(q, k):
                return [_dot_nt(q[:, c], k[:, c]) for c in heads]

            def attend(g, sc, v):
                out = []
                for x, c in zip(sc, heads):
                    x = jnp.where(mask, x * scale, NEG)
                    e = jnp.exp(x - jnp.max(x, axis=-1, keepdims=True))
                    p = e / jnp.sum(e, axis=-1, keepdims=True)
                    o = _dot(p, v[:, c]).astype(BF16)
                    at = g * A_GROUP * DH + c.start
                    u[_rows(S + at // D * ROWS + s * rest, rest), at % D:at % D + DH] = (
                        o[A_PASS:])
                    out.append(o[:A_PASS])
                return out

            early = [_dot(h[:, :D // 2], group_weight(w, 0, 0, D // 2)) for w in (wq, wk, wv)]
            q, k, v = (
                with_rest(m, 0, _dot(h[:, D // 2:], group_weight(w, 0, D // 2, D)) + early[m])
                for m, w in enumerate((wq, wk, wv)))
            o = []
            for g in range(1, n_groups):
                q_next = with_rest(0, g, _dot(h, group_weight(wq, g)))
                sc = scores(q, k)
                k_next = with_rest(1, g, _dot(h, group_weight(wk, g)))
                v_next = with_rest(2, g, _dot(h, group_weight(wv, g)))
                o += attend(g - 1, sc, v)
                q, k, v = q_next, k_next, v_next
            sc = scores(q, k)
            split = H // 2
            y = _dot(jnp.concatenate(o[:split], axis=1), _bf16(woa[:split * DH // 2, :]))
            o += attend(n_groups - 1, sc, v)
            y = _dot(jnp.concatenate(o[split:], axis=1), _bf16(woa[split * DH // 2:, :])) + y
            oa[s] = y[M:].astype(BF16)
            return y[:M]

        def a_step(i, carry):
            memory = mem[...]
            for j in range(A_UNROLL):
                memory = segment(i * A_UNROLL + j, memory)
            mem[...] = memory
            for j in range(A_UNROLL):
                s = i * A_UNROLL + j
                pltpu.make_async_copy(
                    oa.at[s], out_hbm.at[_rows(s * seg, head, seg), 0:D], oa_sem).start()
            return carry

        def out_step(i, carry):
            rows = _rows(jnp.minimum(i, n_rows) * ROWS, ROWS)

            def emit(cols, y):
                y = y + rest_acc[:, cols]
                rest_acc[:, cols] = jnp.where(i >= n_rows, y, 0.0)
                staged[rows, cols] = y.astype(BF16)

            block = jnp.maximum(i - (n_rows - 1), 0)
            a = quadrants(u, i * ROWS)
            dense(a, _left_sums(a).get, wo.at[_rows(block * (D // 2), D // 2)], emit,
                  (2, 6, 3, 1, 5, 7, 4))

            @pl.when(i < n_rows)
            def _():
                pltpu.make_async_copy(
                    staged.at[rows], out_hbm.at[rows, D:2 * D], ob_sem).start()

            return carry

        for t in range(n_tiles):
            vb[t, 0:B_PAD, :] = jnp.broadcast_to(vb[t, B_PAD:B_PAD + 1, :], (B_PAD, LANES))
        ao_copy(0).wait()
        mem_copy(0).wait()
        mem[...] = mem_raw[...].astype(F32)
        lax.fori_loop(0, n_groups, rest_step, 0)
        lax.fori_loop(0, n_seg // A_UNROLL, a_step, 0)
        lax.fori_loop(0, n_rest + n_rows, out_step, 0)

        @pl.loop(0, n_seg)
        def _(s):
            pltpu.make_async_copy(
                staged.at[_rows(S + s * rest, rest)],
                out_hbm.at[_rows(s * seg + head, rest), 0:D], rest_sem).start()

        pltpu.make_async_copy(oa, oa, oa_sem).wait()
        pltpu.make_async_copy(staged.at[:S], staged.at[:S], ob_sem).wait()
        pltpu.make_async_copy(staged.at[S:], staged.at[S:], rest_sem).wait()

    pl.run_scoped(
        finish,
        pltpu.VMEM((3, n_groups, ROWS, A_GROUP * DH), F32),
        pltpu.VMEM((ROWS, D), F32),
        pltpu.VMEM((n_rest * ROWS + S, D), BF16),
        pltpu.VMEM((n_seg, head, D), BF16),
        pltpu.VMEM((ROWS + S, D), BF16),
    )


@functools.partial(jax.jit, static_argnames=("A_seg_len",))
def pallas_concat_heads__memory_aug_recurrent_mem_tr__sliding_local_dilated__prompt_kernel(
    A_x: jax.Array,
    A_mem0: jax.Array,
    A_Wq: jax.Array,
    A_Wk: jax.Array,
    A_Wv: jax.Array,
    A_Wo: jax.Array,
    A_seg_len: int,
    B_x: jax.Array,
    B_wqkv: jax.Array,
    B_wo: jax.Array,
):
    batch, S, D = A_x.shape
    _, H, DH = A_Wq.shape
    M = A_mem0.shape[1]
    seg = int(A_seg_len)
    assert batch == 1 and B_x.shape == A_x.shape
    assert DH == LANES and D == 8 * LANES and D // B_HEADS == 32
    assert S % (seg * A_UNROLL) == 0 and S % ROWS == 0
    assert S // seg * (M + seg - A_PASS) == ROWS

    head_words = pltpu.VMEM((H * (D // 2 + SKEW) + D // 2 + 32, DH), U32)

    out = pl.pallas_call(
        functools.partial(_kernel, seg=seg),
        out_shape=jax.ShapeDtypeStruct((S, 2 * D), BF16),
        in_specs=[pl.BlockSpec(memory_space=pl.ANY)] * 9,
        out_specs=pl.BlockSpec(memory_space=pl.ANY),
        scratch_shapes=[
            head_words, head_words, head_words,
            pltpu.VMEM(((H * DH + D) // 2, D), U32),
            pltpu.VMEM((H * DH, D), BF16),
            pltpu.VMEM((S, D), BF16),
            pltpu.VMEM((M, D), BF16),
            pltpu.VMEM((M, D), F32),
            pltpu.VMEM((7, ROWS // 4, D // 2), U32),
            pltpu.VMEM((D // LANES, B_PAD + S, LANES), F32),
            pltpu.VMEM((2, D // LANES, B_PAD + S, LANES), F32),
            pltpu.VMEM((8, LANES), I32),
            pltpu.SemaphoreType.DMA((14 * (S // ROWS) + 6,)),
        ],
        compiler_params=pltpu.CompilerParams(
            vmem_limit_bytes=126 * 1024 * 1024,
            flags={"XLA_TPU_EVENLY_DISTRIBUTE_CRITICAL_NODES": True}),
        name="concat_heads",
    )(
        A_x.reshape(S, D), A_mem0.reshape(M, D), A_Wq, A_Wk, A_Wv,
        A_Wo.reshape(H * DH, D), B_x.reshape(S, D), B_wqkv, B_wo,
    )
    return out.reshape(batch, S, 2 * D)
```

```python
import functools

import jax
import jax.numpy as jnp
from jax import lax
import jax.experimental.pallas as pl
import jax.experimental.pallas.tpu as pltpu

LANES = 128
NEG = -1000000000.0

B_HEADS = 32
B_TAPS = 8
B_DIL = 2
B_PAD = 16

A_GROUP = 4
A_UNROLL = 2
A_PASS = 32
ROWS = 512
SKEW = 8

F32 = jnp.float32
BF16 = jnp.bfloat16
U32 = jnp.uint32
I32 = jnp.int32


def _dot(a, b):
    return jnp.dot(a, b, preferred_element_type=F32)


def _dot_nt(a, b):
    return lax.dot_general(a, b, (((1,), (1,)), ((), ())), preferred_element_type=F32)


def _bf16(words):
    return pltpu.bitcast(words, BF16)


def _words(halves):
    return pltpu.bitcast(halves, U32)


def _rows(start, size, align=None):
    if not isinstance(start, int):
        start = pl.multiple_of(start, size if align is None else align)
    return pl.ds(start, size)


def _add(a, b):
    return (a.astype(F32) + b.astype(F32)).astype(BF16)


def _sub(a, b):
    return (a.astype(F32) - b.astype(F32)).astype(BF16)


def _left_sums(a):
    a11, a12, a21, a22 = a(0, 0), a(0, 1), a(1, 0), a(1, 1)
    return {1: _add(a11, a22), 2: _add(a21, a22), 5: _add(a11, a12),
            6: _sub(a21, a11), 7: _sub(a12, a22)}


_PRODUCTS = {
    1: (lambda b: _add(b(0, 0), b(1, 1)), ((0, 1), (3, 1))),
    2: (lambda b: b(0, 0), ((2, 1), (3, -1))),
    3: (lambda b: _sub(b(0, 1), b(1, 1)), ((1, 1), (3, 1))),
    4: (lambda b: _sub(b(1, 0), b(0, 0)), ((0, 1), (2, 1))),
    5: (lambda b: b(1, 1), ((0, -1), (1, 1))),
    6: (lambda b: _add(b(0, 0), b(0, 1)), ((3, 1),)),
    7: (lambda b: _add(b(1, 0), b(1, 1)), ((0, 1),)),
}


def _strassen(left, b, each, order):
    c = [None] * 4
    signs = [1] * 4
    for n in order:
        right, uses = _PRODUCTS[n]
        y = _dot(left(n), right(b))
        each(y)
        for q, sign in uses:
            if c[q] is None:
                c[q], signs[q] = y, sign
            elif sign < 0:
                c[q] = c[q] - y
            else:
                c[q], signs[q] = (y + c[q] if signs[q] > 0 else y - c[q]), 1
    return jnp.concatenate(
        [jnp.concatenate(c[:2], axis=1), jnp.concatenate(c[2:], axis=1)], axis=0)


def _swap_blocks(xs, axis, unit, zero):
    n = len(xs)
    size = xs[0].shape[axis]
    pos = ((lax.broadcasted_iota(I32, zero.shape, axis) | zero) // unit) % n
    pos = jnp.tile(pos, (xs[0].shape[0] // zero.shape[0], xs[0].shape[1] // zero.shape[1]))
    xs = [pltpu.roll(x, t * unit, axis) if t else x for t, x in enumerate(xs)]
    out = []
    for j in range(n):
        y = xs[0]
        for t in range(1, n):
            y = jnp.where(pos == (j + t) % n, xs[t], y)
        out.append(y)
    return [pltpu.roll(y, size - j * unit, axis) if j else y for j, y in enumerate(out)]


def _kernel(
    xa_hbm, mem_hbm, wq_hbm, wk_hbm, wv_hbm, woa_hbm, xb_hbm, wqkv_hbm, wob_hbm,
    out_hbm,
    wq, wk, wv, wo, woa_raw, xa, mem_raw, mem, xa_left, kb, vqb, zeros, sems,
    *, seg,
):
    S, D = xa.shape
    _, H, DH = wq_hbm.shape
    M = mem.shape[0]
    L = M + seg
    n_seg = S // seg
    head = A_PASS - M
    rest = seg - head
    pitch = D // 2 + SKEW
    n_tiles = D // LANES
    n_rows = S // ROWS
    n_groups = H // A_GROUP
    n_rest = H * DH // D
    pair = 2 * LANES
    vb, qb = vqb.at[0], vqb.at[1]
    woa = wo.at[D // 2:]

    sem_ids = iter(range(sems.shape[0]))

    def chunked_copy(src, dst, n):
        rows = src.shape[0] // n
        base = [next(sem_ids) for _ in range(n)][0]
        return lambda i: pltpu.make_async_copy(
            src.at[_rows(i * rows, rows)], dst.at[_rows(i * rows, rows)], sems.at[base + i])

    ao_sem = [next(sem_ids) for _ in range(2)][0]
    xa_copy = chunked_copy(xa_hbm, xa, 4 * n_rows)
    mem_copy = chunked_copy(mem_hbm, mem_raw, 1)
    oa_sem = sems.at[next(sem_ids)]
    ob_sem = sems.at[next(sem_ids)]
    rest_sem = sems.at[next(sem_ids)]

    def pack_b_cols(raw, dst, first, rows):
        xs = [_words(raw[_rows(first, rows), t * LANES:(t + 1) * LANES])
              for t in range(n_tiles)]
        for j, x in enumerate(_swap_blocks(xs, 1, 4, jnp.zeros((8, LANES), I32))):
            dst[_rows(first // 2, rows // 2), j * LANES:(j + 1) * LANES] = x

    def pack_b_out(raw, cols, part, zero):
        g, th, jh = part // 4, part // 2 % 2, part % 2
        xs = [_words(raw[pl.ds((4 * th + t) * 128 + g * 32 + jh * 16, 16), cols])
              for t in range(4)]
        for j, x in enumerate(_swap_blocks(xs, 0, 2, zero)):
            wo[pl.ds((4 * jh + j) * 64 + g * 16 + th * 8, 8), cols] = x

    def pack_a_heads(raw, dst, first, rows, zero):
        half = jnp.tile((zero | 16).astype(U32), (H // 16, 1))
        for r in range(rows // 2):
            at = first // 2 + r
            a = _words(raw[2 * at])
            b = _words(raw[2 * at + 1])
            dst[pl.ds(at, H // 2, stride=pitch), :] = (a & 0xFFFF) | (b << half)
            dst[pl.ds(H // 2 * pitch + at, H // 2, stride=pitch), :] = (a >> half) | (
                b & jnp.uint32(0xFFFF0000))

    def head_weight(w, g, j, lo, hi):
        first = g * (A_GROUP * pitch) + j * pitch + lo // 2
        return _bf16(w[_rows(first, (hi - lo) // 2, 8), :])

    def group_weight(w, g, lo=0, hi=D):
        return jnp.concatenate([head_weight(w, g, j, lo, hi) for j in range(A_GROUP)], axis=1)

    def quadrants(x, first):
        return lambda i, j: x[_rows(first + i * (ROWS // 2), ROWS // 2),
                              j * D // 2:(j + 1) * D // 2]

    def dense(a, sums, w, emit, order, side=()):
        per = ROWS // 16
        slots = (D // pair * 7 - 1) * per
        queue = [(j * slots // len(side), job) for j, job in enumerate(side)]
        seen = [0]

        def each(y):
            seen[0] += per
            while queue and queue[0][0] < seen[0]:
                at, job = queue.pop(0)
                r = at % per * 8
                job(pltpu.bitcast(y[r:r + 8, :LANES], I32) & zeros[...])

        for c in range(0, D, pair):
            emit(slice(c, c + pair), _strassen(
                lambda n: a(n - 3, n - 3) if n in (3, 4) else sums(n),
                lambda i, j: _bf16(
                    w[i * D // 4:(i + 1) * D // 4, c + j * LANES:c + (j + 1) * LANES]),
                each, order))

    def project_b(wq_raw, wk_raw, wv_raw, bq_raw, bk_raw, bv_raw, wob_raw, bk, bvq,
                  xb, xb_left):
        xb_copy = chunked_copy(xb_hbm, xb, n_rows)
        bq_copy = chunked_copy(wqkv_hbm.at[:, 0:D], bq_raw, n_rows)
        bk_copy = chunked_copy(wqkv_hbm.at[:, D:2 * D], bk_raw, n_rows)
        bv_copy = chunked_copy(wqkv_hbm.at[:, 2 * D:3 * D], bv_raw, n_rows)
        bo_copy = chunked_copy(wob_hbm, wob_raw, 1)
        a_copies = [
            chunked_copy(src, dst, 2 * n_rows)
            for src, dst in ((wq_hbm, wq_raw), (wk_hbm, wk_raw), (wv_hbm, wv_raw))
        ] + [xa_copy, lambda i: xa_copy(2 * n_rows + i)]

        def store_in(dst, i):
            def emit(cols, y):
                for t in range(2):
                    dst[cols.start // LANES + t, _rows(B_PAD + i * ROWS, ROWS, 8), :] = (
                        y[:, t * LANES:(t + 1) * LANES])

            return emit

        def k_step(i, carry):
            xb_copy(i).wait()
            a = quadrants(xb, i * ROWS)
            sums = _left_sums(a)
            for j, n in enumerate(sums):
                xb_left[i, j] = _words(sums[n])

            def emit(cols, y):
                store_in(kb, i)(cols, y)
                if cols.start == 0:
                    bv_copy(i).wait()
                    bq_copy(i).wait()
                    rows = D // n_rows
                    for raw, dst in ((bv_raw, bvq.at[0]), (bq_raw, bvq.at[1])):
                        for r in range(0, rows, 16):
                            pack_b_cols(raw, dst, i * rows + r, 16)

            dense(a, sums.get, bk, emit, (6, 2, 3, 5, 7, 1, 4))
            return carry

        def vq_step(i, carry):
            steps = 2 * n_rows
            for copy in a_copies:
                copy(i).wait()

            def rest_operands(_):
                per = n_seg // 2 // steps

                def quadrant(a, b):
                    return jnp.concatenate([
                        xa[_rows(((a * steps + i) * per + s) * seg + head, rest),
                           b * D // 2:(b + 1) * D // 2].astype(F32)
                        for s in range(per)], axis=0)

                terms = _left_sums(quadrant)
                terms[3] = quadrant(0, 0).astype(BF16)
                terms[4] = quadrant(1, 1).astype(BF16)
                n = per * rest // 2
                for j in range(1, 8):
                    xa_left[j - 1, _rows(i * n, n), :] = _words(terms[j])

            n = D // steps
            side = [functools.partial(pack_b_out, wob_raw, _rows(i * n, n), part)
                    for part in range(16)]
            side += [functools.partial(pack_a_heads, raw, dst, i * n + r, 4)
                     for raw, dst in ((wq_raw, wq), (wk_raw, wk), (wv_raw, wv))
                     for r in range(0, n, 4)]
            which, block = i // n_rows, i % n_rows
            dense(quadrants(xb, block * ROWS),
                  lambda n: _bf16(xb_left[block, (1, 2, 5, 6, 7).index(n)]),
                  bvq.at[which], store_in(vqb.at[which], block), (6, 2, 3, 1, 5, 7, 4),
                  side + [rest_operands])
            return carry

        for i in range(n_rows):
            bk_copy(i).start()
        for i in range(n_rows):
            xb_copy(i).start()
            bv_copy(i).start()
            bq_copy(i).start()
        zeros[...] = jnp.zeros(zeros.shape, I32)
        for t in range(n_tiles):
            kb[t, 0:B_PAD, :] = jnp.zeros((B_PAD, LANES), F32)
        for i in range(n_rows):
            bk_copy(i).wait()
            rows = D // n_rows
            pack_b_cols(bk_raw, bk, i * rows, rows)
        bo_copy(0).start()
        mem_copy(0).start()
        for i in range(n_rows):
            for copy in a_copies:
                copy(i).start()
        lax.fori_loop(0, n_rows, k_step, 0)
        for i in range(n_rows, 2 * n_rows):
            for copy in a_copies:
                copy(i).start()
        for slot in range(H):
            source = slot % (H // 2) * 2 + slot // (H // 2)
            pltpu.make_async_copy(
                woa_hbm.at[_rows(source * DH, DH)], woa_raw.at[_rows(slot * DH, DH)],
                sems.at[ao_sem + slot // (H // 2)]).start()
        bo_copy(0).wait()
        lax.fori_loop(0, 2 * n_rows, vq_step, 0)

    head_raw = pltpu.VMEM((D, H, DH), BF16)
    square_raw = pltpu.VMEM((D, D), BF16)
    pl.run_scoped(
        project_b, head_raw, head_raw, head_raw, square_raw, square_raw, square_raw,
        square_raw, pltpu.VMEM((D // 2, D), U32), pltpu.VMEM((2, D // 2, D), U32),
        pltpu.VMEM((S, D), BF16), pltpu.VMEM((n_rows, 5, ROWS // 4, D // 2), U32))

    def window_attention(r0, near_start):
        scale = (D // B_HEADS) ** -0.5
        lane = lax.broadcasted_iota(I32, (8, LANES), 1)
        row = lax.broadcasted_iota(I32, (8, LANES), 0)
        taps = [pl.ds(B_PAD + r0 - B_DIL * w, 8) for w in range(B_TAPS)]
        qs = [qb[t, taps[0], :] for t in range(n_tiles)]
        sums = []
        for tap in taps:
            x = qs[0] * kb[0, tap, :]
            for t in range(1, n_tiles):
                x = x + qs[t] * kb[t, tap, :]
            sums.append(x)
        for k in (1, 2):
            sums = [x + jnp.where((lane & k) != 0, pltpu.roll(x, k, 1),
                                  pltpu.roll(x, LANES - k, 1)) for x in sums]
        logits = [x * scale for x in sums]
        if near_start:
            logits = [jnp.where(row + r0 >= B_DIL * w, x, NEG) for w, x in enumerate(logits)]
        top = functools.reduce(jnp.maximum, logits)
        e = [jnp.exp(x - top) for x in logits]
        inv = 1.0 / functools.reduce(jnp.add, e)
        p = [x * inv for x in e]
        tiles = []
        for t in range(n_tiles):
            o = p[0] * vb[t, taps[0], :]
            for w in range(1, B_TAPS):
                o = o + p[w] * vb[t, taps[w], :]
            tiles.append(o)
        return jnp.concatenate(tiles, axis=1)

    def finish(rest_qkv, rest_acc, u, oa, staged):
        def rest_step(g, carry):
            @pl.when(g % (n_groups // 2) == 0)
            def _():
                half = g // (n_groups // 2)
                part = woa_raw.at[_rows(half * (H * DH // 2), H * DH // 2)]
                pltpu.make_async_copy(part, part, sems.at[ao_sem + half]).wait()

            rows = S // n_groups
            base = pl.multiple_of(g * rows, rows)
            pieces = rows // 8
            products = 3 * (A_GROUP * DH // pair) * 7
            seen = [0]
            done = []

            def each(_):
                seen[0] += 1
                while len(done) < min(pieces, (pieces + 2) * seen[0] // (products - 4)):
                    r = 8 * len(done)
                    done.append(window_attention(base + r, r < B_PAD))
                    if r % 16:
                        u[pl.ds(base + (r - 8), 16), :] = jnp.concatenate(
                            done[-2:], axis=0).astype(BF16)

            for m, w in enumerate((wq, wk, wv)):
                for c in range(0, A_GROUP * DH, pair):
                    rest_qkv[m, g, :, c:c + pair] = _strassen(
                        lambda n: _bf16(xa_left[n - 1]),
                        lambda i, j: head_weight(
                            w, g, c // DH + j, i * D // 2, (i + 1) * D // 2),
                        each, (2, 6, 3, 7, 1, 4, 5))
            for j in range(A_GROUP):
                slot = g * A_GROUP + j
                woa[_rows(slot * (DH // 2), DH // 2), :] = _words(
                    woa_raw[_rows(slot * DH, DH), :])
            n = ROWS // n_groups
            rest_acc[_rows(g * n, n), :] = jnp.zeros((n, D), F32)
            return carry

        def segment(s, memory):
            scale = DH ** -0.5
            row = lax.broadcasted_iota(I32, (L, L), 0)
            col = lax.broadcasted_iota(I32, (L, L), 1)
            mask = (row < M) | (row >= col)
            tokens = xa[_rows(s * seg, seg), :].astype(F32)
            h = jnp.concatenate([memory, tokens[:head]], axis=0).astype(BF16)
            heads = [slice(j * DH, (j + 1) * DH) for j in range(A_GROUP)]

            def with_rest(m, g, y):
                return jnp.concatenate([y, rest_qkv[m, g, _rows(s * rest, rest), :]], axis=0)

            def scores(q, k):
                return [_dot_nt(q[:, c], k[:, c]) for c in heads]

            def attend(g, sc, v):
                out = []
                for x, c in zip(sc, heads):
                    x = jnp.where(mask, x * scale, NEG)
                    e = jnp.exp(x - jnp.max(x, axis=-1, keepdims=True))
                    p = e / jnp.sum(e, axis=-1, keepdims=True)
                    o = _dot(p, v[:, c]).astype(BF16)
                    at = g * A_GROUP * DH + c.start
                    u[_rows(S + at // D * ROWS + s * rest, rest), at % D:at % D + DH] = (
                        o[A_PASS:])
                    out.append(o[:A_PASS])
                return out

            early = [_dot(h[:, :D // 2], group_weight(w, 0, 0, D // 2)) for w in (wq, wk, wv)]
            q, k, v = (
                with_rest(m, 0, _dot(h[:, D // 2:], group_weight(w, 0, D // 2, D)) + early[m])
                for m, w in enumerate((wq, wk, wv)))
            o = []
            for g in range(1, n_groups):
                q_next = with_rest(0, g, _dot(h, group_weight(wq, g)))
                sc = scores(q, k)
                k_next = with_rest(1, g, _dot(h, group_weight(wk, g)))
                v_next = with_rest(2, g, _dot(h, group_weight(wv, g)))
                o += attend(g - 1, sc, v)
                q, k, v = q_next, k_next, v_next
            sc = scores(q, k)
            split = H // 2
            y = _dot(jnp.concatenate(o[:split], axis=1), _bf16(woa[:split * DH // 2, :]))
            o += attend(n_groups - 1, sc, v)
            y = _dot(jnp.concatenate(o[split:], axis=1), _bf16(woa[split * DH // 2:, :])) + y
            oa[s] = y[M:].astype(BF16)
            return y[:M]

        def a_step(i, carry):
            memory = mem[...]
            for j in range(A_UNROLL):
                memory = segment(i * A_UNROLL + j, memory)
            mem[...] = memory
            for j in range(A_UNROLL):
                s = i * A_UNROLL + j
                pltpu.make_async_copy(
                    oa.at[s], out_hbm.at[_rows(s * seg, head, seg), 0:D], oa_sem).start()
            return carry

        def out_step(i, carry):
            rows = _rows(jnp.minimum(i, n_rows) * ROWS, ROWS)

            def emit(cols, y):
                y = y + rest_acc[:, cols]
                rest_acc[:, cols] = jnp.where(i >= n_rows, y, 0.0)
                staged[rows, cols] = y.astype(BF16)

            block = jnp.maximum(i - (n_rows - 1), 0)
            a = quadrants(u, i * ROWS)
            dense(a, _left_sums(a).get, wo.at[_rows(block * (D // 2), D // 2)], emit,
                  (2, 6, 3, 1, 5, 7, 4))

            @pl.when(i < n_rows)
            def _():
                pltpu.make_async_copy(
                    staged.at[rows], out_hbm.at[rows, D:2 * D], ob_sem).start()

            return carry

        for t in range(n_tiles):
            vb[t, 0:B_PAD, :] = jnp.broadcast_to(vb[t, B_PAD:B_PAD + 1, :], (B_PAD, LANES))
        mem_copy(0).wait()
        mem[...] = mem_raw[...].astype(F32)
        lax.fori_loop(0, n_groups, rest_step, 0)
        lax.fori_loop(0, n_seg // A_UNROLL, a_step, 0)
        lax.fori_loop(0, n_rest + n_rows, out_step, 0)

        @pl.loop(0, n_seg)
        def _(s):
            pltpu.make_async_copy(
                staged.at[_rows(S + s * rest, rest)],
                out_hbm.at[_rows(s * seg + head, rest), 0:D], rest_sem).start()

        pltpu.make_async_copy(oa, oa, oa_sem).wait()
        pltpu.make_async_copy(staged.at[:S], staged.at[:S], ob_sem).wait()
        pltpu.make_async_copy(staged.at[S:], staged.at[S:], rest_sem).wait()

    pl.run_scoped(
        finish,
        pltpu.VMEM((3, n_groups, ROWS, A_GROUP * DH), F32),
        pltpu.VMEM((ROWS, D), F32),
        pltpu.VMEM((n_rest * ROWS + S, D), BF16),
        pltpu.VMEM((n_seg, head, D), BF16),
        pltpu.VMEM((ROWS + S, D), BF16),
    )


@functools.partial(jax.jit, static_argnames=("A_seg_len",))
def pallas_concat_heads__memory_aug_recurrent_mem_tr__sliding_local_dilated__prompt_kernel(
    A_x: jax.Array,
    A_mem0: jax.Array,
    A_Wq: jax.Array,
    A_Wk: jax.Array,
    A_Wv: jax.Array,
    A_Wo: jax.Array,
    A_seg_len: int,
    B_x: jax.Array,
    B_wqkv: jax.Array,
    B_wo: jax.Array,
):
    batch, S, D = A_x.shape
    _, H, DH = A_Wq.shape
    M = A_mem0.shape[1]
    seg = int(A_seg_len)
    assert batch == 1 and B_x.shape == A_x.shape
    assert DH == LANES and D == 8 * LANES and D // B_HEADS == 32
    assert S % (seg * A_UNROLL) == 0 and S % ROWS == 0
    assert S // seg * (M + seg - A_PASS) == ROWS

    head_words = pltpu.VMEM((H * (D // 2 + SKEW) + D // 2 + 32, DH), U32)

    out = pl.pallas_call(
        functools.partial(_kernel, seg=seg),
        out_shape=jax.ShapeDtypeStruct((S, 2 * D), BF16),
        in_specs=[pl.BlockSpec(memory_space=pl.ANY)] * 9,
        out_specs=pl.BlockSpec(memory_space=pl.ANY),
        scratch_shapes=[
            head_words, head_words, head_words,
            pltpu.VMEM(((H * DH + D) // 2, D), U32),
            pltpu.VMEM((H * DH, D), BF16),
            pltpu.VMEM((S, D), BF16),
            pltpu.VMEM((M, D), BF16),
            pltpu.VMEM((M, D), F32),
            pltpu.VMEM((7, ROWS // 4, D // 2), U32),
            pltpu.VMEM((D // LANES, B_PAD + S, LANES), F32),
            pltpu.VMEM((2, D // LANES, B_PAD + S, LANES), F32),
            pltpu.VMEM((8, LANES), I32),
            pltpu.SemaphoreType.DMA((14 * (S // ROWS) + 7,)),
        ],
        compiler_params=pltpu.CompilerParams(
            vmem_limit_bytes=126 * 1024 * 1024,
            flags={"XLA_TPU_EVENLY_DISTRIBUTE_CRITICAL_NODES": True}),
        name="concat_heads",
    )(
        A_x.reshape(S, D), A_mem0.reshape(M, D), A_Wq, A_Wk, A_Wv,
        A_Wo.reshape(H * DH, D), B_x.reshape(S, D), B_wqkv, B_wo,
    )
    return out.reshape(batch, S, 2 * D)
```
